```python
import jax
import jax.numpy as jnp

def _softmax(x, axis=-1):
    return jax.nn.softmax(x, axis=axis)
def _gelu(x):
    return jax.nn.gelu(x, approximate=True)
def _silu(x):
    return jax.nn.silu(x)
def _sigmoid(x):
    return jax.nn.sigmoid(x)
def _layernorm(x, axis=-1, eps=1e-5):
    m = jnp.mean(x, axis=axis, keepdims=True)
    v = jnp.var(x, axis=axis, keepdims=True)
    return (x - m) / jnp.sqrt(v + eps)
def _scatter_add(tgt, idx, src, axis=0):
    return tgt.at[idx].add(src)
def _segment_sum(src, seg, n):
    return jax.ops.segment_sum(src, seg, n)
class _Rng:
    def __init__(self, key):
        self._k = key
    def _next(self):
        self._k, sub = jax.random.split(self._k)
        return sub
    def normal(self, shape):
        return jax.random.normal(self._next(), shape, dtype=jnp.bfloat16)
    def randint(self, lo, hi, shape):
        return jax.random.randint(self._next(), shape, lo, hi, dtype=jnp.int32)
    def uniform(self, shape, lo=0.0, hi=1.0):
        return jax.random.uniform(self._next(), shape, jnp.bfloat16, lo, hi)
    def permutation(self, n):
        return jax.random.permutation(self._next(), n)


kernel_name = 'interleave_layers__sliding_block_cached__glu_gated_swiglu__decode'

def setup_inputs():
    _rng = _Rng(jax.random.key(int.from_bytes(__import__("os").urandom(4), "little")))
    _w = (lambda a: (lambda t: t.astype(jnp.bfloat16) if jnp.issubdtype(t.dtype, jnp.floating) else t)(jnp.asarray(a)))
    def _A_setup():
        B, Sq, D = 1, 1, 640
        Hq, Hkv, Sk, Dh = 32, 32, 32768, 192
        assert Hq % Hkv == 0, (Hq, Hkv)
        return {
            "x": _w((lambda *s: _rng.normal(s) * 0.05)(B, Sq, D)),
            "k_cache": _w((lambda *s: _rng.normal(s) * 0.05)(B, Hkv, Sk, Dh)),
            "v_cache": _w((lambda *s: _rng.normal(s) * 0.05)(B, Hkv, Sk, Dh)),
            "wq": _w((lambda *s: _rng.normal(s) * 0.05)(D, Hq * Dh) * (D ** -0.5)),
            "wo": _w((lambda *s: _rng.normal(s) * 0.05)(Hq * Dh, D) * ((Hq * Dh) ** -0.5)),
        }
    _A_in = _A_setup()

    def _B_setup():
        B, S, D, F = 1, 1, 640, 1536
        return {
            "x": _w((lambda *s: _rng.normal(s) * 0.05)(B, S, D)),
            "w1": _w((lambda *s: _rng.normal(s) * 0.05)(D, F) * (2.0 / D) ** 0.5),
            "w3": _w((lambda *s: _rng.normal(s) * 0.05)(D, F) * (2.0 / D) ** 0.5),
            "w2": _w((lambda *s: _rng.normal(s) * 0.05)(F, D) * (2.0 / F) ** 0.5),
        }
    _B_in = _B_setup()

    return {
        "A_x": _A_in["x"],
        "A_k_cache": _A_in["k_cache"],
        "A_v_cache": _A_in["v_cache"],
        "A_wq": _A_in["wq"],
        "A_wo": _A_in["wo"],
        "B_x": _B_in["x"],
        "B_w1": _B_in["w1"],
        "B_w3": _B_in["w3"],
        "B_w2": _B_in["w2"],
    }

def reference(A_x, A_k_cache, A_v_cache, A_wq, A_wo, B_x, B_w1, B_w3, B_w2):
    def _A_ref(x, k_cache, v_cache, wq, wo):
        B, Sq, D = x.shape
        Hq, Dh = 32, 192
        Hkv, Sk = k_cache.shape[1], k_cache.shape[2]
        W = min(4096, max(256, Sk // 4))
        rep = Hq // Hkv
        q = (lambda x, *d: x.transpose(*d))((x @ wq).reshape(B, Sq, Hq, Dh), 0, 2, 1, 3)
        k = jnp.repeat(k_cache[:, :, Sk - W:, :], rep, axis=1)
        v = jnp.repeat(v_cache[:, :, Sk - W:, :], rep, axis=1)
        scores = jnp.einsum("bhqd,bhkd->bhqk", q, k) * (Dh ** -0.5)
        p = _softmax(scores, axis=-1)
        o = jnp.einsum("bhqk,bhkd->bhqd", p, v)
        return (lambda x, *d: x.transpose(*d))(o, 0, 2, 1, 3).reshape(B, Sq, Hq * Dh) @ wo

    def _B_ref(x, w1, w3, w2):
        gate = jnp.einsum("bsd,df->bsf", x, w1)
        up = jnp.einsum("bsd,df->bsf", x, w3)
        h = _silu(gate) * up
        out = jnp.einsum("bsf,fd->bsd", h, w2)
        return out

    x = A_x
    x = x + _A_ref(_layernorm(x, axis=-1), A_k_cache, A_v_cache, A_wq, A_wo)
    x = x + _B_ref(_layernorm(x, axis=-1), B_w1, B_w3, B_w2)
    x = x + _A_ref(_layernorm(x, axis=-1), A_k_cache, A_v_cache, A_wq, A_wo)
    x = x + _B_ref(_layernorm(x, axis=-1), B_w1, B_w3, B_w2)
    return x
```

```python
import jax
import jax.numpy as jnp
import numpy as np
from jax import lax
from jax.experimental import pallas as pl
from jax.experimental.pallas import tpu as pltpu

D = 640
H = 32
DH = 192
SK = 32768
W = min(4096, max(256, SK // 4))
F = 1536
EPS = 1e-5

NP = H // 2
NC = W // 128
TP = 2 * DH // 16
DC = D // 128
FC = F // 128
KV_GROUPS = 4
W2_SPLIT = (0, 8, 11, 12)

BF16 = jnp.bfloat16
F32 = jnp.float32
U32 = jnp.uint32


def _tile(words):
    return pltpu.bitcast(words.reshape(64, 128), BF16)


def _mm(lhs_words, tile):
    lhs = pltpu.bitcast(lhs_words, BF16)
    return jnp.dot(lhs, tile, preferred_element_type=F32)[:8]


def _pack(rows8):
    both = jnp.concatenate([rows8, rows8], axis=0).astype(BF16)
    return pltpu.bitcast(both, U32)


def _layernorm(x):
    m = jnp.sum(x, axis=1, keepdims=True) * (1.0 / D)
    d = x - m
    v = jnp.sum(d * d, axis=1, keepdims=True) * (1.0 / D)
    return d * lax.rsqrt(v + EPS)


def _same_head(a, op):
    a = op(a, pltpu.roll(a, 2, 0))
    return op(a, pltpu.roll(a, 4, 0))


def _kernel(
    x_hbm, k_hbm, v_hbm, wq_hbm, wo_hbm, w1_hbm, w3_hbm, w2_hbm,
    o_ref,
    xb, kb16, vb16, wqb16, wob16, w1b16, w3b16, w2b16,
    xl, ql, sa, sb, pb, ab, ol, yb, hl, sems,
):
    kb, vb, wqb, wob, w1b, w3b, w2b = (
        r.bitcast(U32) for r in (kb16, vb16, wqb16, wob16, w1b16, w3b16, w2b16)
    )

    def retiled(src, dst, sem):
        return [
            pltpu.make_async_copy(src.at[:, par], dst.at[:, :, pl.ds(8 * par, 8), :], sem)
            for par in range(2)
        ]

    n = NP * TP // KV_GROUPS
    c0 = SK // 128 - NC
    cp_x = [pltpu.make_async_copy(x_hbm, xb, sems.at[0])]
    cp_wq = retiled(wq_hbm, wqb16, sems.at[1])
    cp_k, cp_v = [], []
    for g in range(KV_GROUPS):
        rows = pl.ds(g * n, n)
        cp_k.append(retiled(k_hbm.at[rows, :, pl.ds(c0, NC)], kb16.at[rows], sems.at[2 + 2 * g]))
        cp_v.append(retiled(v_hbm.at[rows, :, pl.ds(c0, NC)], vb16.at[rows], sems.at[3 + 2 * g]))
    s0 = 2 + 2 * KV_GROUPS
    cp_wo = [pltpu.make_async_copy(wo_hbm, wob16, sems.at[s0])]
    cp_w1 = retiled(w1_hbm, w1b16, sems.at[s0 + 1])
    cp_w3 = retiled(w3_hbm, w3b16, sems.at[s0 + 2])
    cp_w2 = []
    for j, (f0, f1) in enumerate(zip(W2_SPLIT[:-1], W2_SPLIT[1:])):
        rows = pl.ds(8 * f0, 8 * (f1 - f0))
        cp_w2.append([pltpu.make_async_copy(w2_hbm.at[rows], w2b16.at[rows], sems.at[s0 + 3 + j])])

    order = cp_wq + cp_x
    for g in range(KV_GROUPS):
        order += cp_k[g] + cp_v[g]
    order += cp_wo + cp_w1 + cp_w3 + sum(cp_w2, [])
    for c in order:
        c.start()

    def wait(copies):
        for c in copies:
            c.wait()

    def set_lhs(x):
        xl[...] = _pack(_layernorm(x))

    def stage_q(i):
        for j in range(3):
            q = None
            for t in range(DC):
                r = _mm(xl[:, 128 * t:128 * (t + 1)], _tile(wqb[8 * t:8 * (t + 1), 3 * i + j]))
                q = r if q is None else q + r
            if j == 1:
                row = lax.broadcasted_iota(jnp.int32, q.shape, 0)
                col = lax.broadcasted_iota(jnp.int32, q.shape, 1)
                q = jnp.where((row & 1) == (col >> 6), q, 0.0)
            ql[i, j] = _pack(q)

    def stage_k(i, slot):
        q = [ql[i, j] for j in range(3)]
        for c in range(NC):
            u = (2 * c) % 8
            r = [_mm(q[j], _tile(kb[pl.ds(TP * i + 8 * j, 8), c])) for j in range(3)]
            sa[slot, 2 * c:2 * c + 1, :] = r[0][u:u + 1]
            sb[slot, 2 * c:2 * c + 2, :] = r[1][u:u + 2]
            sa[slot, 2 * c + 1:2 * c + 2, :] = r[2][u + 1:u + 2]

    def stage_softmax(slot):
        s = (sa[slot] + sb[slot]) * (DH ** -0.5)
        s = s.reshape(2 * NC // 8, 8, 128)
        m = jnp.max(_same_head(jnp.max(s, axis=0), jnp.maximum), axis=1, keepdims=True)
        e = jnp.exp(s - m[None])
        l = jnp.sum(_same_head(jnp.sum(e, axis=0), jnp.add), axis=1, keepdims=True)
        pb[slot] = (e * (1.0 / l)[None]).reshape(2 * NC, 128)

    def stage_v(i, slot, group=4):
        for t0 in range(0, TP, group):
            e = t0 // (TP // 2)
            lo, hi = [None] * group, [None] * group
            for c in range(NC):
                p = jnp.broadcast_to(pb[slot, 2 * c + e:2 * c + e + 1, :], (8, 128))
                for u in range(group):
                    w = vb[TP * i + t0 + u, c]
                    a = pltpu.bitcast(w << 16, F32) * p
                    b = pltpu.bitcast(w & np.uint32(0xFFFF0000), F32) * p
                    lo[u] = a if c == 0 else lo[u] + a
                    hi[u] = b if c == 0 else hi[u] + b
            for u in range(group):
                ab[slot, pl.ds(16 * (t0 + u), 8, stride=2), :] = lo[u]
                ab[slot, pl.ds(16 * (t0 + u) + 1, 8, stride=2), :] = hi[u]

    def stage_o(i, slot):
        for j in range(3):
            t = ab[slot, 128 * j:128 * (j + 1), :].T
            o = jnp.sum(t.reshape(16, 8, 128), axis=0)
            o = o + pltpu.roll(o, 1, 0)
            ol[i, j] = _pack(_same_head(o, jnp.add))

    def halves(ref, rows, c):
        return jnp.concatenate(
            [ref[rows, 4 * c:4 * c + 4, :], ref[rows, 20 + 4 * c:24 + 4 * c, :]], axis=1
        )

    def stage_wo_first(i):
        for j in range(3):
            rows = pl.ds(TP * i + 8 * j, 8)
            ws = [halves(wob, rows, c) for c in range(DC)]
            for c in range(DC):
                wob[rows, 8 * c:8 * c + 8, :] = ws[c]
                yb[0:8, 128 * c:128 * (c + 1)] += _mm(ol[i, j], _tile(ws[c]))

    def stage_wo(i):
        for j in range(3):
            b = 3 * i + j
            for c in range(DC):
                r = _mm(ol[i, j], _tile(wob[8 * b:8 * b + 8, 8 * c:8 * c + 8, :]))
                yb[b:b + 1, 128 * c:128 * (c + 1)] = r[b % 8:b % 8 + 1]

    def ffn_up():
        for f in range(FC):
            gu = []
            for w in (w1b, w3b):
                acc = None
                for t in range(DC):
                    r = _mm(xl[:, 128 * t:128 * (t + 1)], _tile(w[8 * t:8 * (t + 1), f]))
                    acc = r if acc is None else acc + r
                gu.append(acc)
            g, u = gu
            hl[f] = _pack(g * (1.0 / (1.0 + jnp.exp(-g))) * u)

    def ffn_down(x, f0, f1):
        cols = [x[:, 128 * c:128 * (c + 1)] for c in range(DC)]
        for f in range(f0, f1):
            for c in range(DC):
                cols[c] = cols[c] + _mm(hl[f], _tile(halves(w2b, slice(8 * f, 8 * f + 8), c)))
        return jnp.concatenate(cols, axis=1)

    def loop(lo, hi, fn):
        def body(i, carry):
            fn(i)
            return carry

        lax.fori_loop(lo, hi, body, 0)

    wait(cp_x)
    x = jnp.broadcast_to(xb[...].astype(F32), (8, D))
    set_lhs(x)
    wait(cp_wq)
    loop(0, NP, stage_q)
    per = NP // KV_GROUPS

    def attend(i):
        for g in range(KV_GROUPS):
            @pl.when(i == g * per)
            def _():
                wait(cp_k[g] + cp_v[g])

        stage_k(i, 0)
        stage_softmax(0)
        stage_v(i, 0)
        stage_o(i, 0)

    loop(0, NP, attend)
    yb[0:8] = x
    wait(cp_wo)
    loop(0, NP, stage_wo_first)
    x = yb[0:8]
    set_lhs(x)
    wait(cp_w1 + cp_w3)
    ffn_up()
    for j, (f0, f1) in enumerate(zip(W2_SPLIT[:-1], W2_SPLIT[1:])):
        wait(cp_w2[j])
        x = ffn_down(x, f0, f1)

    set_lhs(x)
    stage_q(0)
    for i in range(NP + 2):
        if i + 1 < NP:
            stage_q(i + 1)
        if i < NP:
            stage_k(i, i)
            stage_softmax(i)
            stage_v(i, i)
            stage_o(i, i)
        if i >= 2:
            stage_wo(i - 2)
    y = jnp.sum(yb[...].reshape(H * DH // 1024, 8, D), axis=0)
    y = y + pltpu.roll(y, 1, 0)
    x = x + _same_head(y, jnp.add)
    set_lhs(x)
    ffn_up()
    x = ffn_down(x, 0, FC)
    o_ref[...] = x[0:1].astype(o_ref.dtype)


def _groups(w):
    r, c = w.shape
    return w.reshape(r // 16, 2, 8, c // 128, 128).transpose(0, 1, 3, 2, 4)


@jax.jit
def pallas_interleave_layers__sliding_block_cached__glu_gated_swiglu__decode_kernel(
    A_x: jax.Array,
    A_k_cache: jax.Array,
    A_v_cache: jax.Array,
    A_wq: jax.Array,
    A_wo: jax.Array,
    B_x: jax.Array,
    B_w1: jax.Array,
    B_w3: jax.Array,
    B_w2: jax.Array,
):
    del B_x

    def cache(c):
        return _groups(jnp.swapaxes(c, 2, 3).reshape(H * DH, SK))

    def flat(w):
        return _groups(w).reshape(w.shape[0] // 16, 2 * DC * 8, 128)

    out = pl.pallas_call(
        _kernel,
        out_shape=jax.ShapeDtypeStruct((1, D), A_x.dtype),
        in_specs=[pl.BlockSpec(memory_space=pl.ANY)] * 8,
        scratch_shapes=[
            pltpu.VMEM((1, D), BF16),
            pltpu.VMEM((NP * TP, NC, 16, 128), BF16),
            pltpu.VMEM((NP * TP, NC, 16, 128), BF16),
            pltpu.VMEM((D // 16, H * DH // 128, 16, 128), BF16),
            pltpu.VMEM((H * DH // 16, 2 * DC * 8, 128), BF16),
            pltpu.VMEM((D // 16, FC, 16, 128), BF16),
            pltpu.VMEM((D // 16, FC, 16, 128), BF16),
            pltpu.VMEM((F // 16, 2 * DC * 8, 128), BF16),
            pltpu.VMEM((8, D), U32),
            pltpu.VMEM((NP, 3, 8, 128), U32),
            pltpu.VMEM((NP, 2 * NC, 128), F32),
            pltpu.VMEM((NP, 2 * NC, 128), F32),
            pltpu.VMEM((NP, 2 * NC, 128), F32),
            pltpu.VMEM((NP, 2 * DH, 128), F32),
            pltpu.VMEM((NP, 3, 8, 128), U32),
            pltpu.VMEM((H * DH // 128, D), F32),
            pltpu.VMEM((FC, 8, 128), U32),
            pltpu.SemaphoreType.DMA((5 + 2 * KV_GROUPS + len(W2_SPLIT) - 1,)),
        ],
        compiler_params=pltpu.CompilerParams(vmem_limit_bytes=128 * 1024 * 1024),
        name="interleave_decode",
    )(
        A_x.reshape(1, D),
        cache(A_k_cache),
        cache(A_v_cache),
        _groups(A_wq),
        flat(A_wo),
        _groups(B_w1),
        _groups(B_w3),
        flat(B_w2),
    )
    return out.reshape(1, 1, D)
```

```python
import jax
import jax.numpy as jnp
import numpy as np
from jax import lax
from jax.experimental import pallas as pl
from jax.experimental.pallas import tpu as pltpu

D = 640
H = 32
DH = 192
SK = 32768
W = min(4096, max(256, SK // 4))
F = 1536
EPS = 1e-5

NP = H // 2
NC = W // 128
TP = 2 * DH // 16
DC = D // 128
FC = F // 128
KV_SPLIT = (16, 12, 8, 4, 2, 1, 0)
WO_PARTS = 8
IN_FLIGHT = 3
W2_SPLIT = (0, 8, 11, 12)
V_GROUP = 4
V_ON_MXU = 64

BF16 = jnp.bfloat16
F32 = jnp.float32
U32 = jnp.uint32


def _tile(words):
    return pltpu.bitcast(words.reshape(64, 128), BF16)


def _mm(lhs_words, tile):
    lhs = pltpu.bitcast(lhs_words, BF16)
    return jnp.dot(lhs, tile, preferred_element_type=F32)[:8]


def _pack(rows8):
    both = jnp.concatenate([rows8, rows8], axis=0).astype(BF16)
    return pltpu.bitcast(both, U32)


def _layernorm(x):
    m = jnp.sum(x, axis=1, keepdims=True) * (1.0 / D)
    d = x - m
    v = jnp.sum(d * d, axis=1, keepdims=True) * (1.0 / D)
    return d * lax.rsqrt(v + EPS)


def _same_head(a, op):
    a = op(a, pltpu.roll(a, 2, 0))
    return op(a, pltpu.roll(a, 4, 0))


def _own_head(a, j):
    row = lax.broadcasted_iota(jnp.int32, a.shape, 0)
    col = lax.broadcasted_iota(jnp.int32, a.shape, 1)
    return jnp.where((row & 1) == ((col >> 6) + j >> 1), a, 0.0)


VPU_CHUNKS = [min(max(NP * NC - V_ON_MXU - NC * i, 0), NC) for i in range(NP)]


def _kernel(
    x_hbm, k_hbm, v_hbm, wq_hbm, wo_hbm, w1_hbm, w3_hbm, w2_hbm,
    o_ref,
    xb, big, xl, ol, yb, hl, sems, fence, slots,
):
    kb16, vb16, wqb16, wob16, w1b16, w3b16, w2b16 = big
    kb, vb, wqb, wob, w1b, w3b, w2b = (r.bitcast(U32) for r in big)

    def retiled(src, dst, *sem):
        return [
            pltpu.make_async_copy(src.at[:, par], dst.at[:, :, pl.ds(8 * par, 8), :], sem[-par])
            for par in range(2)
        ]

    free = (sems.at[n] for n in range(sems.shape[0]))
    cp_x = [pltpu.make_async_copy(x_hbm, xb, next(free))]
    cp_wq = retiled(wq_hbm, wqb16, next(free))
    cp_kv = []
    for hi, lo in zip(KV_SPLIT[:-1], KV_SPLIT[1:]):
        rows, sem = pl.ds(TP * lo, TP * (hi - lo)), next(free)
        window = pl.ds(SK // 128 - NC, NC)
        cp_kv.append(
            retiled(k_hbm.at[rows, :, window], kb16.at[rows], sem)
            + retiled(v_hbm.at[rows, :, window], vb16.at[rows], sem)
        )
    for c in cp_wq + cp_x + sum(cp_kv, []):
        c.start()

    late = []
    for n in range(WO_PARTS):
        rows = pl.ds(n * NP * TP // WO_PARTS, NP * TP // WO_PARTS)
        late.append(pltpu.make_async_copy(wo_hbm.at[rows], wob16.at[rows], next(free)))
    for src, dst in ((w1_hbm, w1b16), (w3_hbm, w3b16)):
        late += retiled(src, dst, next(free), next(free))
    for f0, f1 in zip(W2_SPLIT[:-1], W2_SPLIT[1:]):
        rows = pl.ds(8 * f0, 8 * (f1 - f0))
        late.append(pltpu.make_async_copy(w2_hbm.at[rows], w2b16.at[rows], next(free)))

    def wait(copies):
        for c in copies:
            c.wait()

    def wait_late(n):
        late[n].wait()
        if n + IN_FLIGHT < len(late):
            late[n + IN_FLIGHT].start(priority=1)

    def set_lhs(x):
        xl[...] = _pack(_layernorm(x))

    def stage_q(i, s):
        for j in range(3):
            for t in range(DC):
                w = _tile(wqb[8 * t:8 * (t + 1), 3 * i + j])
                s["r"][j, t] = _mm(xl[:, 128 * t:128 * (t + 1)], w)

    def finish_q(s):
        for j in range(3):
            q = jnp.sum(s["r"][j], axis=0)
            s["q"][j] = _pack(_own_head(q, j) if j == 1 else q)

    def stage_k(i, s):
        for c in range(NC):
            u = (2 * c) % 8
            r = [_mm(s["q"][j], _tile(kb[pl.ds(TP * i + 8 * j, 8), c])) for j in range(3)]
            s["a"][2 * c:2 * c + 1, :] = r[0][u:u + 1]
            s["b"][2 * c:2 * c + 2, :] = r[1][u:u + 2]
            s["a"][2 * c + 1:2 * c + 2, :] = r[2][u + 1:u + 2]

    def spread(ref, a):
        for r in range(a.shape[0]):
            ref[8 * r:8 * r + 8, :] = jnp.broadcast_to(a[r:r + 1], (8, 128))

    def softmax_lanes(s, chunks):
        z = (s["a"][...] + s["b"][...]) * (DH ** -0.5)
        z = z.reshape(2 * NC // 8, 8, 128)
        m = _same_head(jnp.max(z, axis=0), jnp.maximum)
        e = jnp.exp(z - m[None])
        l = _same_head(jnp.sum(e, axis=0), jnp.add)
        s["m"][0], s["m"][1] = m, l
        e = e.reshape(2 * NC, 128)
        spread(s["p"], e[:2 * chunks])
        if chunks < NC:
            s["e"][...] = e

    def row_max(s):
        s["M"][...] = jnp.broadcast_to(jnp.max(s["m"][0], axis=1, keepdims=True), (8, 128))

    def weigh_lanes(s, chunks):
        f = jnp.exp(s["m"][0] - s["M"][...])
        s["l"][...] = f * s["m"][1]
        if chunks > 0:
            for e in range(2):
                rows = slice(e * DH, (e + 1) * DH)
                s["u"][rows, :] = s["o"][rows, :] * f[e:e + 1]
        if chunks < NC:
            p = s["e"][...].reshape(-1, 8, 128) * f[None]
            w = pltpu.bitcast(p.reshape(2 * NC, 128).astype(BF16), U32)
            spread(s["w"].at[8 * chunks:], w[chunks:])

    def stage_v(i, s, t0, chunks):
        e = t0 // (TP // 2)
        lo, hi = [None] * V_GROUP, [None] * V_GROUP
        for c in range(chunks):
            p = s["p"][8 * (2 * c + e):8 * (2 * c + e + 1), :]
            for u in range(V_GROUP):
                w = vb[TP * i + t0 + u, c]
                a = pltpu.bitcast(w << 16, F32) * p
                b = pltpu.bitcast(w & np.uint32(0xFFFF0000), F32) * p
                lo[u] = a if c == 0 else lo[u] + a
                hi[u] = b if c == 0 else hi[u] + b
        for u in range(V_GROUP):
            s["o"][pl.ds(16 * (t0 + u), 8, stride=2), :] = lo[u]
            s["o"][pl.ds(16 * (t0 + u) + 1, 8, stride=2), :] = hi[u]

    def flip_o(s, chunks):
        s["L"][...] = jnp.broadcast_to(jnp.sum(s["l"][...], axis=1, keepdims=True), (8, 128))
        for j in range(3 if chunks > 0 else 0):
            s["t"][j] = s["u"][128 * j:128 * (j + 1), :].T

    def stage_o(s, chunks):
        out, scale = [], 1.0 / s["L"][...]
        for j in range(3):
            o = None
            if chunks > 0:
                o = jnp.sum(s["t"][j].reshape(16, 8, 128), axis=0)
            if chunks < NC:
                part = jnp.sum(s["z"][j, 2 * chunks:, :].reshape(-1, 8, 128), axis=0)
                part = _own_head(part, j)
                o = part if o is None else o + part
            inv = _own_head(scale, j)
            o = o * (inv + pltpu.roll(inv, 1, 0))
            o = _same_head(o, jnp.add)
            out.append(_pack(o + pltpu.roll(o, 1, 0)))
        return out

    def transpose_v(n):
        i, c = n // NC, n % NC
        for j in range(3):
            rows = pl.ds(TP * i + 8 * j, 8)
            vb[rows, c] = pltpu.bitcast(_tile(vb[rows, c]).T, U32).reshape(8, 8, 128)

    def stage_v_mxu(i, s, chunks):
        for c in range(chunks, NC):
            u = (2 * c) % 8
            for j in range(3):
                r = _mm(s["w"][8 * c:8 * c + 8, :], _tile(vb[pl.ds(TP * i + 8 * j, 8), c]))
                s["z"][j, 2 * c:2 * c + 2, :] = r[u:u + 2]

    def halves(ref, rows, c):
        return jnp.concatenate(
            [ref[rows, 4 * c:4 * c + 4, :], ref[rows, 20 + 4 * c:24 + 4 * c, :]], axis=1
        )

    def stage_wo_first(i):
        for j in range(3):
            rows = pl.ds(TP * i + 8 * j, 8)
            ws = [halves(wob, rows, c) for c in range(DC)]
            for c in range(DC):
                wob[rows, 8 * c:8 * c + 8, :] = ws[c]
                yb[c, 0] += _mm(ol[i, j], _tile(ws[c]))

    def stage_wo(i, e):
        for j in range(3):
            n = 3 * e + j
            for c in range(DC):
                w = _tile(wob[pl.ds(TP * i + 8 * j, 8), 8 * c:8 * c + 8, :])
                yb[c, i // 2, n:n + 1, :] = _mm(slots[e]["y"][j], w)[n:n + 1]

    def ffn_up():
        for f in range(FC):
            gu = []
            for w in (w1b, w3b):
                acc = None
                for t in range(DC):
                    r = _mm(xl[:, 128 * t:128 * (t + 1)], _tile(w[8 * t:8 * (t + 1), f]))
                    acc = r if acc is None else acc + r
                gu.append(acc)
            g, u = gu
            hl[f] = _pack(g * (1.0 / (1.0 + jnp.exp(-g))) * u)

    def ffn_down(x, f0, f1):
        cols = [x[:, 128 * c:128 * (c + 1)] for c in range(DC)]
        for f in range(f0, f1):
            for c in range(DC):
                cols[c] = cols[c] + _mm(hl[f], _tile(halves(w2b, slice(8 * f, 8 * f + 8), c)))
        return jnp.concatenate(cols, axis=1)

    def loop(lo, hi, fn):
        def body(i, carry):
            fn(i)
            return carry

        lax.fori_loop(lo, hi, body, 0)

    wait(cp_x)
    x = jnp.broadcast_to(xb[...].astype(F32), (8, D))
    set_lhs(x)
    wait(cp_wq)

    def attend(n):
        i = NP - 1 - n
        for g, hi in enumerate(KV_SPLIT[:-1]):
            @pl.when(i == hi - 1)
            def _():
                wait(cp_kv[g])
                if g == len(cp_kv) - 2:
                    for c in late[:IN_FLIGHT]:
                        c.start(priority=1)

        s = slots[0]
        stage_q(i, s)
        finish_q(s)
        stage_k(i, s)
        softmax_lanes(s, NC)
        for t0 in range(0, TP, V_GROUP):
            stage_v(i, s, t0, NC)
        row_max(s)
        weigh_lanes(s, NC)
        flip_o(s, NC)
        for j, o in enumerate(stage_o(s, NC)):
            ol[i, j] = o
        loop(jnp.maximum(NC * i, NP * NC - V_ON_MXU), NC * (i + 1), transpose_v)

    loop(0, NP, attend)
    for c in range(DC):
        yb[c, 0] = x[:, 128 * c:128 * (c + 1)]

    def project(i):
        for n in range(WO_PARTS):
            pl.when(i == n * NP // WO_PARTS)(lambda: wait_late(n))
        stage_wo_first(i)

    loop(0, NP, project)
    x = jnp.concatenate([yb[c, 0] for c in range(DC)], axis=1)
    set_lhs(x)
    yb[...] = jnp.zeros(yb.shape, F32)
    for name in "mMoulLty":
        slots[1][name][...] = slots[0][name][...] if name != "y" else ol[0]
    slots[0]["y"][...] = ol[0]
    for n in range(4):
        wait_late(WO_PARTS + n)
    ffn_up()
    for j, (f0, f1) in enumerate(zip(W2_SPLIT[:-1], W2_SPLIT[1:])):
        wait_late(WO_PARTS + 4 + j)
        x = ffn_down(x, f0, f1)

    set_lhs(x)

    def finish_o(s, chunks):
        for j, o in enumerate(stage_o(s, chunks)):
            s["y"][j] = o

    def barrier():
        pl.semaphore_wait(fence, 0)

    def step(i, e):
        this, other = slots[e], slots[1 - e]
        glue = [
            lambda: finish_q(other),
            lambda: finish_o(other, NC),
            lambda: weigh_lanes(other, NC),
            lambda: softmax_lanes(other, NC),
        ]
        for t0 in range(0, TP, V_GROUP):
            stage_v(i, this, t0, NC)
            if glue:
                glue.pop(0)()
        stage_k(i + 2, this)
        stage_q(jnp.minimum(i + 4, NP - 1), this)
        stage_wo(jnp.maximum(i - 4, e), e)
        row_max(this)
        flip_o(this, NC)

    def two_steps(n):
        step(2 * n, 0)
        barrier()
        step(2 * n + 1, 1)

    even, odd = slots
    for i, s in enumerate(slots):
        stage_q(i, s)
        finish_q(s)
    stage_k(0, even)
    softmax_lanes(even, NC)
    stage_k(1, odd)
    stage_q(2, even)
    finish_q(even)
    stage_q(3, odd)
    loop(0, NP // 2 - 1, two_steps)

    stage_wo(NP - 6, 0)
    finish_o(odd, NC)
    flip_o(even, NC)
    finish_o(even, NC)
    weigh_lanes(odd, NC)
    flip_o(odd, NC)
    softmax_lanes(even, 0)
    softmax_lanes(odd, 0)
    stage_wo(NP - 5, 1)
    stage_wo(NP - 4, 0)
    finish_o(odd, NC)
    for s in slots:
        row_max(s)
        weigh_lanes(s, 0)
        flip_o(s, 0)
    stage_v_mxu(NP - 2, even, 0)
    stage_wo(NP - 3, 1)
    stage_v_mxu(NP - 1, odd, 0)
    for e, s in enumerate(slots):
        finish_o(s, 0)
        stage_wo(NP - 2 + e, e)
    y = jnp.concatenate([jnp.sum(yb[c], axis=0) for c in range(DC)], axis=1)
    y = y + pltpu.roll(y, 1, 0)
    x = x + _same_head(y, jnp.add)
    set_lhs(x)
    ffn_up()
    x = ffn_down(x, 0, FC)
    o_ref[...] = x[0:1].astype(o_ref.dtype)


def _groups(w):
    r, c = w.shape
    return w.reshape(r // 16, 2, 8, c // 128, 128).transpose(0, 1, 3, 2, 4)


@jax.jit
def pallas_interleave_layers__sliding_block_cached__glu_gated_swiglu__decode_kernel(
    A_x: jax.Array,
    A_k_cache: jax.Array,
    A_v_cache: jax.Array,
    A_wq: jax.Array,
    A_wo: jax.Array,
    B_x: jax.Array,
    B_w1: jax.Array,
    B_w3: jax.Array,
    B_w2: jax.Array,
):
    del B_x

    def cache(c):
        return _groups(jnp.swapaxes(c, 2, 3).reshape(H * DH, SK))

    def flat(w):
        return _groups(w).reshape(w.shape[0] // 16, 2 * DC * 8, 128)

    slot = {
        "r": pltpu.VMEM((3, DC, 8, 128), F32),
        "q": pltpu.VMEM((3, 8, 128), U32),
        "a": pltpu.VMEM((2 * NC, 128), F32),
        "b": pltpu.VMEM((2 * NC, 128), F32),
        "m": pltpu.VMEM((2, 8, 128), F32),
        "p": pltpu.VMEM((16 * NC, 128), F32),
        "e": pltpu.VMEM((2 * NC, 128), F32),
        "M": pltpu.VMEM((8, 128), F32),
        "o": pltpu.VMEM((2 * DH, 128), F32),
        "u": pltpu.VMEM((2 * DH, 128), F32),
        "l": pltpu.VMEM((8, 128), F32),
        "L": pltpu.VMEM((8, 128), F32),
        "t": pltpu.VMEM((3, 128, 128), F32),
        "w": pltpu.VMEM((8 * NC, 128), U32),
        "z": pltpu.VMEM((3, 2 * NC, 128), F32),
        "y": pltpu.VMEM((3, 8, 128), U32),
    }
    out = pl.pallas_call(
        _kernel,
        out_shape=jax.ShapeDtypeStruct((1, D), A_x.dtype),
        in_specs=[pl.BlockSpec(memory_space=pl.ANY)] * 8,
        scratch_shapes=[
            pltpu.VMEM((1, D), BF16),
            [
                pltpu.VMEM((NP * TP, NC, 16, 128), BF16),
                pltpu.VMEM((NP * TP, NC, 16, 128), BF16),
                pltpu.VMEM((D // 16, H * DH // 128, 16, 128), BF16),
                pltpu.VMEM((H * DH // 16, 2 * DC * 8, 128), BF16),
                pltpu.VMEM((D // 16, FC, 16, 128), BF16),
                pltpu.VMEM((D // 16, FC, 16, 128), BF16),
                pltpu.VMEM((F // 16, 2 * DC * 8, 128), BF16),
            ],
            pltpu.VMEM((8, D), U32),
            pltpu.VMEM((NP, 3, 8, 128), U32),
            pltpu.VMEM((DC, NP // 2, 8, 128), F32),
            pltpu.VMEM((FC, 8, 128), U32),
            pltpu.SemaphoreType.DMA((len(KV_SPLIT) + WO_PARTS + len(W2_SPLIT) + 4,)),
            pltpu.SemaphoreType.REGULAR(()),
            [slot] * 2,
        ],
        compiler_params=pltpu.CompilerParams(vmem_limit_bytes=128 * 1024 * 1024),
        name="interleave_decode",
    )(
        A_x.reshape(1, D),
        cache(A_k_cache),
        cache(A_v_cache),
        _groups(A_wq),
        flat(A_wo),
        _groups(B_w1),
        _groups(B_w3),
        flat(B_w2),
    )
    return out.reshape(1, 1, D)
```

```python
import jax
import jax.numpy as jnp
import numpy as np
from jax import lax
from jax.experimental import pallas as pl
from jax.experimental.pallas import tpu as pltpu

D = 640
H = 32
DH = 192
SK = 32768
W = min(4096, max(256, SK // 4))
F = 1536
EPS = 1e-5

NP = H // 2
NC = W // 128
TP = 2 * DH // 16
DC = D // 128
FC = F // 128
KV_SPLIT = (16, 12, 8, 4, 2, 1, 0)
WO_PARTS = 8
IN_FLIGHT = 3
W2_SPLIT = (0, 8, 11, 12)
V_GROUP = 4
WIDE = 5
V_ON_MXU = 0

BF16 = jnp.bfloat16
F32 = jnp.float32
U32 = jnp.uint32


def _tile(words):
    return pltpu.bitcast(words.reshape(64, 128), BF16)


def _mm(lhs_words, tile):
    lhs = pltpu.bitcast(lhs_words, BF16)
    return jnp.dot(lhs, tile, preferred_element_type=F32)[:8]


def _pack(rows8):
    both = jnp.concatenate([rows8, rows8], axis=0).astype(BF16)
    return pltpu.bitcast(both, U32)


def _layernorm(x):
    m = jnp.sum(x, axis=1, keepdims=True) * (1.0 / D)
    d = x - m
    v = jnp.sum(d * d, axis=1, keepdims=True) * (1.0 / D)
    return d * lax.rsqrt(v + EPS)


def _same_head(a, op):
    a = op(a, pltpu.roll(a, 2, 0))
    return op(a, pltpu.roll(a, 4, 0))


def _own_head(a, j):
    row = lax.broadcasted_iota(jnp.int32, a.shape, 0)
    col = lax.broadcasted_iota(jnp.int32, a.shape, 1)
    return jnp.where((row & 1) == ((col >> 6) + j >> 1), a, 0.0)


VPU_CHUNKS = [min(max(NP * NC - V_ON_MXU - NC * i, 0), NC) for i in range(NP)]


def _kernel(
    x_hbm, k_hbm, v_hbm, wq_hbm, wo_hbm, w1_hbm, w3_hbm, w2_hbm,
    o_ref,
    xb, big, vx, xl, ol, yb, hl, sems, fence, slots,
):
    kb16, vb16, wqb16, wob16, w1b16, w3b16, w2b16 = big
    kb, vb, wqb, wob, w1b, w3b, w2b = (r.bitcast(U32) for r in big)

    def retiled(src, dst, *sem):
        return [
            pltpu.make_async_copy(src.at[:, par], dst.at[:, :, pl.ds(8 * par, 8), :], sem[-par])
            for par in range(2)
        ]

    free = (sems.at[n] for n in range(sems.shape[0]))
    cp_x = [pltpu.make_async_copy(x_hbm, xb, next(free))]
    cp_wq = retiled(wq_hbm, wqb16, next(free))
    cp_kv = []
    for hi, lo in zip(KV_SPLIT[:-1], KV_SPLIT[1:]):
        rows, sem = pl.ds(TP * lo, TP * (hi - lo)), next(free)
        window = pl.ds(SK // 128 - NC, NC)
        cp_kv.append(
            retiled(k_hbm.at[rows, :, window], kb16.at[rows], sem)
            + retiled(v_hbm.at[rows, :, window], vb16.at[rows], sem)
        )
    for c in cp_wq + cp_x + sum(cp_kv, []):
        c.start()

    late = []
    for n in range(WO_PARTS):
        rows = pl.ds(n * NP * TP // WO_PARTS, NP * TP // WO_PARTS)
        late.append(pltpu.make_async_copy(wo_hbm.at[rows], wob16.at[rows], next(free)))
    for src, dst in ((w1_hbm, w1b16), (w3_hbm, w3b16)):
        late += retiled(src, dst, next(free), next(free))
    for f0, f1 in zip(W2_SPLIT[:-1], W2_SPLIT[1:]):
        rows = pl.ds(8 * f0, 8 * (f1 - f0))
        late.append(pltpu.make_async_copy(w2_hbm.at[rows], w2b16.at[rows], next(free)))

    def wait(copies):
        for c in copies:
            c.wait()

    def wait_late(n):
        late[n].wait()
        if n + IN_FLIGHT < len(late):
            late[n + IN_FLIGHT].start(priority=1)

    def set_lhs(x):
        xl[...] = _pack(_layernorm(x))

    def stage_q(i, s):
        for j in range(3):
            for t in range(DC):
                w = _tile(wqb[8 * t:8 * (t + 1), 3 * i + j])
                s["r"][j, t] = _mm(xl[:, 128 * t:128 * (t + 1)], w)

    def finish_q(s):
        for j in range(3):
            q = jnp.sum(s["r"][j], axis=0)
            s["q"][j] = _pack(_own_head(q, j) if j == 1 else q)

    def stage_k(i, s):
        for c in range(NC):
            u = (2 * c) % 8
            r = [_mm(s["q"][j], _tile(kb[pl.ds(TP * i + 8 * j, 8), c])) for j in range(3)]
            s["a"][2 * c:2 * c + 1, :] = r[0][u:u + 1]
            s["b"][2 * c:2 * c + 2, :] = r[1][u:u + 2]
            s["a"][2 * c + 1:2 * c + 2, :] = r[2][u + 1:u + 2]

    def spread(ref, a):
        for r in range(0, a.shape[0], 8):
            for u in range(r, r + 8):
                ref[8 * u:8 * u + 8, :] = jnp.broadcast_to(a[u:u + 1], (8, 128))

    def softmax_lanes(s, chunks):
        z = (s["a"][...] + s["b"][...]) * (DH ** -0.5)
        z = z.reshape(2 * NC // 8, 8, 128)
        m = _same_head(jnp.max(z, axis=0), jnp.maximum)
        e = jnp.exp(z - m[None])
        l = _same_head(jnp.sum(e, axis=0), jnp.add)
        s["m"][0], s["m"][1] = m, l
        e = e.reshape(2 * NC, 128)
        spread(s["p"], e[:2 * chunks])
        if chunks < NC:
            s["e"][...] = e

    def row_max(s):
        s["M"][...] = jnp.broadcast_to(jnp.max(s["m"][0], axis=1, keepdims=True), (8, 128))

    def weigh_lanes(s, chunks):
        f = jnp.exp(s["m"][0] - s["M"][...])
        s["l"][...] = f * s["m"][1]
        if chunks > 0:
            for e in range(2):
                rows = slice(e * DH, (e + 1) * DH)
                s["u"][rows, :] = s["o"][rows, :] * f[e:e + 1]
        if chunks < NC:
            p = s["e"][...].reshape(-1, 8, 128) * f[None]
            w = pltpu.bitcast(p.reshape(2 * NC, 128).astype(BF16), U32)
            spread(s["w"].at[8 * chunks:], w[chunks:])

    def stage_v(i, s, t0, chunks, wide):
        e = t0 // (TP // 2)
        lo, hi = [None] * V_GROUP, [None] * V_GROUP
        for c in range(chunks):
            p = s["p"][8 * (2 * c + e):8 * (2 * c + e + 1), :]
            for u in range(V_GROUP):
                w = vb[TP * i + t0 + u, c]
                x = c - (NC - WIDE)
                if wide and x >= 0:
                    a, b = w, vx[TP * i + t0 + u, x]
                else:
                    a, b = w << 16, w & np.uint32(0xFFFF0000)
                    if x >= 0:
                        vb[TP * i + t0 + u, c], vx[TP * i + t0 + u, x] = a, b
                a, b = pltpu.bitcast(a, F32) * p, pltpu.bitcast(b, F32) * p
                lo[u] = a if c == 0 else lo[u] + a
                hi[u] = b if c == 0 else hi[u] + b
        for u in range(V_GROUP):
            s["o"][pl.ds(16 * (t0 + u), 8, stride=2), :] = lo[u]
            s["o"][pl.ds(16 * (t0 + u) + 1, 8, stride=2), :] = hi[u]

    def flip_o(s, chunks):
        s["L"][...] = jnp.broadcast_to(jnp.sum(s["l"][...], axis=1, keepdims=True), (8, 128))
        for j in range(3 if chunks > 0 else 0):
            s["t"][j] = s["u"][128 * j:128 * (j + 1), :].T

    def stage_o(s, chunks):
        out, scale = [], 1.0 / s["L"][...]
        for j in range(3):
            o = None
            if chunks > 0:
                o = jnp.sum(s["t"][j].reshape(16, 8, 128), axis=0)
            if chunks < NC:
                part = jnp.sum(s["z"][j, 2 * chunks:, :].reshape(-1, 8, 128), axis=0)
                part = _own_head(part, j)
                o = part if o is None else o + part
            inv = _own_head(scale, j)
            o = o * (inv + pltpu.roll(inv, 1, 0))
            o = _same_head(o, jnp.add)
            out.append(_pack(o + pltpu.roll(o, 1, 0)))
        return out

    def transpose_v(n):
        i, c = n // NC, n % NC
        for j in range(3):
            rows = pl.ds(TP * i + 8 * j, 8)
            vb[rows, c] = pltpu.bitcast(_tile(vb[rows, c]).T, U32).reshape(8, 8, 128)

    def stage_v_mxu(i, s, chunks):
        for c in range(chunks, NC):
            u = (2 * c) % 8
            for j in range(3):
                r = _mm(s["w"][8 * c:8 * c + 8, :], _tile(vb[pl.ds(TP * i + 8 * j, 8), c]))
                s["z"][j, 2 * c:2 * c + 2, :] = r[u:u + 2]

    def halves(ref, rows, c):
        return jnp.concatenate(
            [ref[rows, 4 * c:4 * c + 4, :], ref[rows, 20 + 4 * c:24 + 4 * c, :]], axis=1
        )

    def stage_wo_first(i):
        for j in range(3):
            rows = pl.ds(TP * i + 8 * j, 8)
            ws = [halves(wob, rows, c) for c in range(DC)]
            for c in range(DC):
                wob[rows, 8 * c:8 * c + 8, :] = ws[c]
                yb[c, 0] += _mm(ol[i, j], _tile(ws[c]))

    def stage_wo(i):
        for b in range(3 * i, 3 * i + 3):
            for c in range(DC):
                r = _mm(ol[i, b % 3], _tile(wob[8 * b:8 * b + 8, 8 * c:8 * c + 8, :]))
                yb[c, b // 8, b % 8:b % 8 + 1, :] = r[b % 8:b % 8 + 1]

    def ffn_up():
        for f in range(FC):
            gu = []
            for w in (w1b, w3b):
                acc = None
                for t in range(DC):
                    r = _mm(xl[:, 128 * t:128 * (t + 1)], _tile(w[8 * t:8 * (t + 1), f]))
                    acc = r if acc is None else acc + r
                gu.append(acc)
            g, u = gu
            hl[f] = _pack(g * (1.0 / (1.0 + jnp.exp(-g))) * u)

    def ffn_down(x, f0, f1):
        cols = [x[:, 128 * c:128 * (c + 1)] for c in range(DC)]
        for f in range(f0, f1):
            for c in range(DC):
                cols[c] = cols[c] + _mm(hl[f], _tile(halves(w2b, slice(8 * f, 8 * f + 8), c)))
        return jnp.concatenate(cols, axis=1)

    def loop(lo, hi, fn):
        def body(i, carry):
            fn(i)
            return carry

        lax.fori_loop(lo, hi, body, 0)

    wait(cp_x)
    x = jnp.broadcast_to(xb[...].astype(F32), (8, D))
    set_lhs(x)
    wait(cp_wq)

    def attend(n):
        i = NP - 1 - n
        for g, hi in enumerate(KV_SPLIT[:-1]):
            @pl.when(i == hi - 1)
            def _():
                wait(cp_kv[g])
                if g == len(cp_kv) - 2:
                    for c in late[:IN_FLIGHT]:
                        c.start(priority=1)

        s = slots[0]
        stage_q(i, s)
        finish_q(s)
        stage_k(i, s)
        softmax_lanes(s, NC)
        for t0 in range(0, TP, V_GROUP):
            stage_v(i, s, t0, NC, 0)
        row_max(s)
        weigh_lanes(s, NC)
        flip_o(s, NC)
        for j, o in enumerate(stage_o(s, NC)):
            ol[i, j] = o
        loop(jnp.maximum(NC * i, NP * NC - V_ON_MXU), NC * (i + 1), transpose_v)

    loop(0, NP, attend)
    for c in range(DC):
        yb[c, 0] = x[:, 128 * c:128 * (c + 1)]

    def project(i):
        for n in range(WO_PARTS):
            pl.when(i == n * NP // WO_PARTS)(lambda: wait_late(n))
        stage_wo_first(i)

    loop(0, NP, project)
    x = jnp.concatenate([yb[c, 0] for c in range(DC)], axis=1)
    set_lhs(x)
    for name in "mMoulLt":
        slots[1][name][...] = slots[0][name][...]
    for n in range(4):
        wait_late(WO_PARTS + n)
    ffn_up()
    for j, (f0, f1) in enumerate(zip(W2_SPLIT[:-1], W2_SPLIT[1:])):
        wait_late(WO_PARTS + 4 + j)
        x = ffn_down(x, f0, f1)

    set_lhs(x)

    def barrier():
        pl.semaphore_wait(fence, 0)

    def finish_o(s, i):
        for j, o in enumerate(stage_o(s, NC)):
            ol[i, j] = o

    def step(i, e, more=2):
        this, other = slots[e], slots[1 - e]
        weigh_lanes(other, NC)
        finish_o(other, jnp.maximum(i - 3, 0))
        if more > 1:
            finish_q(other)
        if more > 0:
            softmax_lanes(other, NC)
        for t0 in range(0, TP, V_GROUP):
            stage_v(i, this, t0, NC, WIDE)
        if more > 1:
            stage_k(i + 2, this)
            stage_q(jnp.minimum(i + 4, NP - 1), this)
        row_max(this)
        flip_o(this, NC)

    def two_steps(n):
        step(2 * n, 0)
        barrier()
        step(2 * n + 1, 1)

    even, odd = slots
    for i, s in enumerate(slots):
        stage_q(i, s)
        finish_q(s)
    stage_k(0, even)
    softmax_lanes(even, NC)
    stage_k(1, odd)
    stage_q(2, even)
    finish_q(even)
    stage_q(3, odd)
    loop(0, NP // 2 - 1, two_steps)
    step(NP - 2, 0, 1)
    for i in range(7):
        stage_wo(i)
    barrier()
    step(NP - 1, 1, 0)
    for i in range(7, NP - 4):
        stage_wo(i)
    barrier()
    finish_o(even, NP - 4)
    finish_o(odd, NP - 3)
    weigh_lanes(odd, NC)
    for i, s in enumerate(slots, NP - 2):
        flip_o(s, NC)
        finish_o(s, i)
    for i in range(NP - 4, NP):
        stage_wo(i)
    y = jnp.concatenate([jnp.sum(yb[c], axis=0) for c in range(DC)], axis=1)
    y = y + pltpu.roll(y, 1, 0)
    x = x + _same_head(y, jnp.add)
    set_lhs(x)
    ffn_up()
    x = ffn_down(x, 0, FC)
    o_ref[...] = x[0:1].astype(o_ref.dtype)


def _groups(w):
    r, c = w.shape
    return w.reshape(r // 16, 2, 8, c // 128, 128).transpose(0, 1, 3, 2, 4)


@jax.jit
def pallas_interleave_layers__sliding_block_cached__glu_gated_swiglu__decode_kernel(
    A_x: jax.Array,
    A_k_cache: jax.Array,
    A_v_cache: jax.Array,
    A_wq: jax.Array,
    A_wo: jax.Array,
    B_x: jax.Array,
    B_w1: jax.Array,
    B_w3: jax.Array,
    B_w2: jax.Array,
):
    del B_x

    def cache(c):
        return _groups(jnp.swapaxes(c, 2, 3).reshape(H * DH, SK))

    def flat(w):
        return _groups(w).reshape(w.shape[0] // 16, 2 * DC * 8, 128)

    slot = {
        "r": pltpu.VMEM((3, DC, 8, 128), F32),
        "q": pltpu.VMEM((3, 8, 128), U32),
        "a": pltpu.VMEM((2 * NC, 128), F32),
        "b": pltpu.VMEM((2 * NC, 128), F32),
        "m": pltpu.VMEM((2, 8, 128), F32),
        "p": pltpu.VMEM((16 * NC, 128), F32),
        "M": pltpu.VMEM((8, 128), F32),
        "o": pltpu.VMEM((2 * DH, 128), F32),
        "u": pltpu.VMEM((2 * DH, 128), F32),
        "l": pltpu.VMEM((8, 128), F32),
        "L": pltpu.VMEM((8, 128), F32),
        "t": pltpu.VMEM((3, 128, 128), F32),
        "y": pltpu.VMEM((3, 8, 128), U32),
    }
    out = pl.pallas_call(
        _kernel,
        out_shape=jax.ShapeDtypeStruct((1, D), A_x.dtype),
        in_specs=[pl.BlockSpec(memory_space=pl.ANY)] * 8,
        scratch_shapes=[
            pltpu.VMEM((1, D), BF16),
            [
                pltpu.VMEM((NP * TP, NC, 16, 128), BF16),
                pltpu.VMEM((NP * TP, NC, 16, 128), BF16),
                pltpu.VMEM((D // 16, H * DH // 128, 16, 128), BF16),
                pltpu.VMEM((H * DH // 16, 2 * DC * 8, 128), BF16),
                pltpu.VMEM((D // 16, FC, 16, 128), BF16),
                pltpu.VMEM((D // 16, FC, 16, 128), BF16),
                pltpu.VMEM((F // 16, 2 * DC * 8, 128), BF16),
            ],
            pltpu.VMEM((NP * TP, WIDE, 8, 128), U32),
            pltpu.VMEM((8, D), U32),
            pltpu.VMEM((NP, 3, 8, 128), U32),
            pltpu.VMEM((DC, 3 * NP // 8, 8, 128), F32),
            pltpu.VMEM((FC, 8, 128), U32),
            pltpu.SemaphoreType.DMA((len(KV_SPLIT) + WO_PARTS + len(W2_SPLIT) + 4,)),
            pltpu.SemaphoreType.REGULAR(()),
            [slot] * 2,
        ],
        compiler_params=pltpu.CompilerParams(vmem_limit_bytes=128 * 1024 * 1024),
        name="interleave_decode",
    )(
        A_x.reshape(1, D),
        cache(A_k_cache),
        cache(A_v_cache),
        _groups(A_wq),
        flat(A_wo),
        _groups(B_w1),
        _groups(B_w3),
        flat(B_w2),
    )
    return out.reshape(1, 1, D)
```

```python
import jax
import jax.numpy as jnp
import numpy as np
from jax import lax
from jax.experimental import pallas as pl
from jax.experimental.pallas import tpu as pltpu

D = 640
H = 32
DH = 192
SK = 32768
W = min(4096, max(256, SK // 4))
F = 1536
EPS = 1e-5

NP = H // 2
NC = W // 128
TP = 2 * DH // 16
DC = D // 128
FC = F // 128
KV_SPLIT = (16, 12, 8, 4, 2, 1, 0)
WO_PARTS = 8
IN_FLIGHT = 3
W2_SPLIT = (0, 8, 11, 12)
V_GROUP = 4
WIDE = 6

BF16 = jnp.bfloat16
F32 = jnp.float32
U32 = jnp.uint32


def _tile(words):
    return pltpu.bitcast(words.reshape(64, 128), BF16)


def _mm(lhs_words, tile):
    lhs = pltpu.bitcast(lhs_words, BF16)
    return jnp.dot(lhs, tile, preferred_element_type=F32)[:8]


def _pack(rows8):
    both = jnp.concatenate([rows8, rows8], axis=0).astype(BF16)
    return pltpu.bitcast(both, U32)


def _layernorm(x):
    m = jnp.sum(x, axis=1, keepdims=True) * (1.0 / D)
    d = x - m
    v = jnp.sum(d * d, axis=1, keepdims=True) * (1.0 / D)
    return d * lax.rsqrt(v + EPS)


def _same_head(a, op):
    a = op(a, pltpu.roll(a, 2, 0))
    return op(a, pltpu.roll(a, 4, 0))


def _own_head(a, j):
    row = lax.broadcasted_iota(jnp.int32, a.shape, 0)
    col = lax.broadcasted_iota(jnp.int32, a.shape, 1)
    return jnp.where((row & 1) == ((col >> 6) + j >> 1), a, 0.0)


def _kernel(
    x_hbm, k_hbm, v_hbm, wq_hbm, wo_hbm, w1_hbm, w3_hbm, w2_hbm,
    o_ref,
    xb, big, vx, xl, ol, yb, hl, sems, fence, slots,
):
    kb16, vb16, wqb16, wob16, w1b16, w3b16, w2b16 = big
    kb, vb, wqb, wob, w1b, w3b, w2b = (r.bitcast(U32) for r in big)

    def retiled(src, dst, *sem):
        return [
            pltpu.make_async_copy(src.at[:, par], dst.at[:, :, pl.ds(8 * par, 8), :], sem[-par])
            for par in range(2)
        ]

    free = (sems.at[n] for n in range(sems.shape[0]))
    cp_x = [pltpu.make_async_copy(x_hbm, xb, next(free))]
    cp_wq = retiled(wq_hbm, wqb16, next(free))
    cp_kv = []
    for hi, lo in zip(KV_SPLIT[:-1], KV_SPLIT[1:]):
        rows, sem = pl.ds(TP * lo, TP * (hi - lo)), next(free)
        window = pl.ds(SK // 128 - NC, NC)
        cp_kv.append(
            retiled(k_hbm.at[rows, :, window], kb16.at[rows], sem)
            + retiled(v_hbm.at[rows, :, window], vb16.at[rows], sem)
        )
    for c in cp_wq + cp_x + sum(cp_kv, []):
        c.start()

    late = []
    for n in range(WO_PARTS):
        rows = pl.ds(n * NP * TP // WO_PARTS, NP * TP // WO_PARTS)
        late.append(pltpu.make_async_copy(wo_hbm.at[rows], wob16.at[rows], next(free)))
    for src, dst in ((w1_hbm, w1b16), (w3_hbm, w3b16)):
        late += retiled(src, dst, next(free), next(free))
    for f0, f1 in zip(W2_SPLIT[:-1], W2_SPLIT[1:]):
        rows = pl.ds(8 * f0, 8 * (f1 - f0))
        late.append(pltpu.make_async_copy(w2_hbm.at[rows], w2b16.at[rows], next(free)))

    def wait(copies):
        for c in copies:
            c.wait()

    def wait_late(n):
        late[n].wait()
        if n + IN_FLIGHT < len(late):
            late[n + IN_FLIGHT].start(priority=1)

    def set_lhs(x):
        xl[...] = _pack(_layernorm(x))

    def stage_q(i, s):
        for j in range(3):
            for t in range(DC):
                w = _tile(wqb[8 * t:8 * (t + 1), 3 * i + j])
                s["r"][j, t] = _mm(xl[:, 128 * t:128 * (t + 1)], w)

    def finish_q(s):
        for j in range(3):
            q = jnp.sum(s["r"][j], axis=0)
            s["q"][j] = _pack(_own_head(q, j) if j == 1 else q)

    def stage_k(i, s):
        for c in range(NC):
            u = (2 * c) % 8
            r = [_mm(s["q"][j], _tile(kb[pl.ds(TP * i + 8 * j, 8), c])) for j in range(3)]
            s["a"][2 * c:2 * c + 1, :] = r[0][u:u + 1]
            s["b"][2 * c:2 * c + 2, :] = r[1][u:u + 2]
            s["a"][2 * c + 1:2 * c + 2, :] = r[2][u + 1:u + 2]

    def softmax_lanes(s):
        z = (s["a"][...] + s["b"][...]) * (DH ** -0.5)
        z = z.reshape(2 * NC // 8, 8, 128)
        m = _same_head(jnp.max(z, axis=0), jnp.maximum)
        e = jnp.exp(z - m[None])
        s["m"][0], s["m"][1] = m, _same_head(jnp.sum(e, axis=0), jnp.add)
        e = e.reshape(2 * NC, 128)
        for r in range(2 * NC):
            s["p"][8 * r:8 * r + 8, :] = jnp.broadcast_to(e[r:r + 1], (8, 128))

    def row_max(s):
        s["M"][...] = jnp.broadcast_to(jnp.max(s["m"][0], axis=1, keepdims=True), (8, 128))

    def stage_v(i, s, wide):
        for t0 in range(0, TP, V_GROUP):
            e = t0 // (TP // 2)
            lo, hi = [None] * V_GROUP, [None] * V_GROUP
            for c in range(NC):
                p = s["p"][8 * (2 * c + e):8 * (2 * c + e + 1), :]
                for u in range(V_GROUP):
                    t, x = TP * i + t0 + u, c - (NC - WIDE)
                    w = vb[t, c]
                    if wide and x >= 0:
                        a, b = w, vx[t, x]
                    else:
                        a, b = w << 16, w & np.uint32(0xFFFF0000)
                        if x >= 0:
                            vb[t, c], vx[t, x] = a, b
                    a, b = pltpu.bitcast(a, F32) * p, pltpu.bitcast(b, F32) * p
                    lo[u] = a if c == 0 else lo[u] + a
                    hi[u] = b if c == 0 else hi[u] + b
            for u in range(V_GROUP):
                s["o"][pl.ds(16 * (t0 + u), 8, stride=2), :] = lo[u]
                s["o"][pl.ds(16 * (t0 + u) + 1, 8, stride=2), :] = hi[u]

    def weigh_lanes(s):
        f = jnp.exp(s["m"][0] - s["M"][...])
        s["l"][...] = f * s["m"][1]
        for e in range(2):
            rows = slice(e * DH, (e + 1) * DH)
            s["u"][rows, :] = s["o"][rows, :] * f[e:e + 1]

    def flip_o(s):
        s["L"][...] = jnp.broadcast_to(jnp.sum(s["l"][...], axis=1, keepdims=True), (8, 128))
        for j in range(0, 2 * DH, 128):
            s["u"][j:j + 128, :] = s["u"][j:j + 128, :].T

    def finish_o(i, s):
        scale = 1.0 / s["L"][...]
        for j in range(3):
            inv = _own_head(scale, j)
            o = jnp.sum(s["u"][128 * j:128 * (j + 1), :].reshape(16, 8, 128), axis=0)
            o = _same_head(o * (inv + pltpu.roll(inv, 1, 0)), jnp.add)
            ol[i, j] = _pack(o + pltpu.roll(o, 1, 0))

    def halves(ref, rows, c):
        return jnp.concatenate(
            [ref[rows, 4 * c:4 * c + 4, :], ref[rows, 20 + 4 * c:24 + 4 * c, :]], axis=1
        )

    def stage_wo_first(i):
        for j in range(3):
            rows = pl.ds(TP * i + 8 * j, 8)
            ws = [halves(wob, rows, c) for c in range(DC)]
            for c in range(DC):
                wob[rows, 8 * c:8 * c + 8, :] = ws[c]
                yb[c, 0] += _mm(ol[i, j], _tile(ws[c]))

    def stage_wo(i):
        for b in range(3 * i, 3 * i + 3):
            for c in range(DC):
                r = _mm(ol[i, b % 3], _tile(wob[8 * b:8 * b + 8, 8 * c:8 * c + 8, :]))
                yb[c, b // 8, b % 8:b % 8 + 1, :] = r[b % 8:b % 8 + 1]

    def ffn_up():
        for f in range(FC):
            gu = []
            for w in (w1b, w3b):
                acc = None
                for t in range(DC):
                    r = _mm(xl[:, 128 * t:128 * (t + 1)], _tile(w[8 * t:8 * (t + 1), f]))
                    acc = r if acc is None else acc + r
                gu.append(acc)
            g, u = gu
            hl[f] = _pack(g * (1.0 / (1.0 + jnp.exp(-g))) * u)

    def ffn_down(x, f0, f1):
        cols = [x[:, 128 * c:128 * (c + 1)] for c in range(DC)]
        for f in range(f0, f1):
            for c in range(DC):
                cols[c] = cols[c] + _mm(hl[f], _tile(halves(w2b, slice(8 * f, 8 * f + 8), c)))
        return jnp.concatenate(cols, axis=1)

    def loop(lo, hi, fn):
        def body(i, carry):
            fn(i)
            return carry

        lax.fori_loop(lo, hi, body, 0)

    wait(cp_x)
    x = jnp.broadcast_to(xb[...].astype(F32), (8, D))
    set_lhs(x)
    wait(cp_wq)

    def attend(n):
        i = NP - 1 - n
        for g, hi in enumerate(KV_SPLIT[:-1]):
            @pl.when(i == hi - 1)
            def _():
                wait(cp_kv[g])
                if g == len(cp_kv) - 2:
                    for c in late[:IN_FLIGHT]:
                        c.start(priority=1)

        s = slots[0]
        stage_q(i, s)
        finish_q(s)
        stage_k(i, s)
        softmax_lanes(s)
        stage_v(i, s, False)
        row_max(s)
        weigh_lanes(s)
        flip_o(s)
        finish_o(i, s)

    loop(0, NP, attend)
    for c in range(DC):
        yb[c, 0] = x[:, 128 * c:128 * (c + 1)]

    def project(i):
        for n in range(WO_PARTS):
            pl.when(i == n * NP // WO_PARTS)(lambda: wait_late(n))
        stage_wo_first(i)

    loop(0, NP, project)
    x = jnp.concatenate([yb[c, 0] for c in range(DC)], axis=1)
    set_lhs(x)
    for name in "mMoulL":
        slots[1][name][...] = slots[0][name][...]
    for n in range(4):
        wait_late(WO_PARTS + n)
    ffn_up()
    for j, (f0, f1) in enumerate(zip(W2_SPLIT[:-1], W2_SPLIT[1:])):
        wait_late(WO_PARTS + 4 + j)
        x = ffn_down(x, f0, f1)

    set_lhs(x)

    def barrier():
        pl.semaphore_wait(fence, 0)

    def step(i, e, more=2):
        this, other = slots[e], slots[1 - e]
        finish_o(jnp.maximum(i - 3, 0), other)
        weigh_lanes(other)
        if more > 1:
            finish_q(other)
        if more > 0:
            softmax_lanes(other)
        stage_v(i, this, True)
        if more > 1:
            stage_k(i + 2, this)
            stage_q(jnp.minimum(i + 4, NP - 1), this)
        row_max(this)
        flip_o(this)

    def two_steps(n):
        step(2 * n, 0)
        barrier()
        step(2 * n + 1, 1)

    even, odd = slots
    for i, s in enumerate(slots):
        stage_q(i, s)
        finish_q(s)
    stage_k(0, even)
    softmax_lanes(even)
    stage_k(1, odd)
    stage_q(2, even)
    finish_q(even)
    stage_q(3, odd)
    loop(0, NP // 2 - 1, two_steps)
    step(NP - 2, 0, 1)
    for i in range(6):
        stage_wo(i)
    barrier()
    step(NP - 1, 1, 0)
    for i in range(6, NP - 4):
        stage_wo(i)
    barrier()
    finish_o(NP - 3, odd)
    weigh_lanes(odd)
    for i, s in enumerate(slots, NP - 2):
        flip_o(s)
        finish_o(i, s)
    for i in range(NP - 4, NP):
        stage_wo(i)
    y = jnp.concatenate([jnp.sum(yb[c], axis=0) for c in range(DC)], axis=1)
    y = y + pltpu.roll(y, 1, 0)
    x = x + _same_head(y, jnp.add)
    set_lhs(x)
    ffn_up()
    x = ffn_down(x, 0, FC)
    o_ref[...] = x[0:1].astype(o_ref.dtype)


def _groups(w):
    r, c = w.shape
    return w.reshape(r // 16, 2, 8, c // 128, 128).transpose(0, 1, 3, 2, 4)


@jax.jit
def pallas_interleave_layers__sliding_block_cached__glu_gated_swiglu__decode_kernel(
    A_x: jax.Array,
    A_k_cache: jax.Array,
    A_v_cache: jax.Array,
    A_wq: jax.Array,
    A_wo: jax.Array,
    B_x: jax.Array,
    B_w1: jax.Array,
    B_w3: jax.Array,
    B_w2: jax.Array,
):
    del B_x

    def cache(c):
        return _groups(jnp.swapaxes(c, 2, 3).reshape(H * DH, SK))

    def flat(w):
        return _groups(w).reshape(w.shape[0] // 16, 2 * DC * 8, 128)

    slot = {
        "r": pltpu.VMEM((3, DC, 8, 128), F32),
        "q": pltpu.VMEM((3, 8, 128), U32),
        "a": pltpu.VMEM((2 * NC, 128), F32),
        "b": pltpu.VMEM((2 * NC, 128), F32),
        "m": pltpu.VMEM((2, 8, 128), F32),
        "p": pltpu.VMEM((16 * NC, 128), F32),
        "M": pltpu.VMEM((8, 128), F32),
        "o": pltpu.VMEM((2 * DH, 128), F32),
        "u": pltpu.VMEM((2 * DH, 128), F32),
        "l": pltpu.VMEM((8, 128), F32),
        "L": pltpu.VMEM((8, 128), F32),
        "y": pltpu.VMEM((3, 8, 128), U32),
    }
    out = pl.pallas_call(
        _kernel,
        out_shape=jax.ShapeDtypeStruct((1, D), A_x.dtype),
        in_specs=[pl.BlockSpec(memory_space=pl.ANY)] * 8,
        scratch_shapes=[
            pltpu.VMEM((1, D), BF16),
            [
                pltpu.VMEM((NP * TP, NC, 16, 128), BF16),
                pltpu.VMEM((NP * TP, NC, 16, 128), BF16),
                pltpu.VMEM((D // 16, H * DH // 128, 16, 128), BF16),
                pltpu.VMEM((H * DH // 16, 2 * DC * 8, 128), BF16),
                pltpu.VMEM((D // 16, FC, 16, 128), BF16),
                pltpu.VMEM((D // 16, FC, 16, 128), BF16),
                pltpu.VMEM((F // 16, 2 * DC * 8, 128), BF16),
            ],
            pltpu.VMEM((NP * TP, WIDE, 8, 128), U32),
            pltpu.VMEM((8, D), U32),
            pltpu.VMEM((NP, 3, 8, 128), U32),
            pltpu.VMEM((DC, 3 * NP // 8, 8, 128), F32),
            pltpu.VMEM((FC, 8, 128), U32),
            pltpu.SemaphoreType.DMA((len(KV_SPLIT) + WO_PARTS + len(W2_SPLIT) + 4,)),
            pltpu.SemaphoreType.REGULAR(()),
            [slot] * 2,
        ],
        compiler_params=pltpu.CompilerParams(vmem_limit_bytes=128 * 1024 * 1024),
        name="interleave_decode",
    )(
        A_x.reshape(1, D),
        cache(A_k_cache),
        cache(A_v_cache),
        _groups(A_wq),
        flat(A_wo),
        _groups(B_w1),
        _groups(B_w3),
        flat(B_w2),
    )
    return out.reshape(1, 1, D)
```

```python
import jax
import jax.numpy as jnp
import numpy as np
from jax import lax
from jax.experimental import pallas as pl
from jax.experimental.pallas import tpu as pltpu

D = 640
H = 32
DH = 192
SK = 32768
W = min(4096, max(256, SK // 4))
F = 1536
EPS = 1e-5

NP = H // 2
NC = W // 128
TP = 2 * DH // 16
DC = D // 128
FC = F // 128
KV_SPLIT = (16, 12, 8, 4, 2, 1, 0)
WO_PARTS = 8
IN_FLIGHT = 3
W2_SPLIT = (0, 8, 11, 12)
V_GROUP = 6
WIDE = 6

BF16 = jnp.bfloat16
F32 = jnp.float32
U32 = jnp.uint32


def _tile(words):
    return pltpu.bitcast(words.reshape(64, 128), BF16)


def _mm(lhs_words, tile):
    lhs = pltpu.bitcast(lhs_words, BF16)
    return jnp.dot(lhs, tile, preferred_element_type=F32)[:8]


def _pack(rows8):
    both = jnp.concatenate([rows8, rows8], axis=0).astype(BF16)
    return pltpu.bitcast(both, U32)


def _same_head(a, op):
    a = op(a, pltpu.roll(a, 2, 0))
    return op(a, pltpu.roll(a, 4, 0))


def _own_head(a, j):
    row = lax.broadcasted_iota(jnp.int32, a.shape, 0)
    col = lax.broadcasted_iota(jnp.int32, a.shape, 1)
    return jnp.where((row & 1) == ((col >> 6) + j >> 1), a, 0.0)


def _kernel(
    x_hbm, k_hbm, v_hbm, wq_hbm, wo_hbm, w1_hbm, w3_hbm, w2_hbm,
    o_ref,
    xb, big, vx, xl, rstd, ol, yb, hl, sems, fence, slots,
):
    kb16, vb16, wqb16, wob16, w1b16, w3b16, w2b16 = big
    kb, vb, wqb, wob, w1b, w3b, w2b = (r.bitcast(U32) for r in big)

    def retiled(src, dst, *sem):
        return [
            pltpu.make_async_copy(src.at[:, par], dst.at[:, :, pl.ds(8 * par, 8), :], sem[-par])
            for par in range(2)
        ]

    free = (sems.at[n] for n in range(sems.shape[0]))
    cp_x = [pltpu.make_async_copy(x_hbm, xb, next(free))]
    cp_wq = retiled(wq_hbm, wqb16, next(free))
    cp_kv = []
    for hi, lo in zip(KV_SPLIT[:-1], KV_SPLIT[1:]):
        rows, sem = pl.ds(TP * lo, TP * (hi - lo)), next(free)
        window = pl.ds(SK // 128 - NC, NC)
        cp_kv.append(
            retiled(k_hbm.at[rows, :, window], kb16.at[rows], sem)
            + retiled(v_hbm.at[rows, :, window], vb16.at[rows], sem)
        )
    for c in cp_wq + cp_x + sum(cp_kv, []):
        c.start()

    late = []
    for n in range(WO_PARTS):
        rows = pl.ds(n * NP * TP // WO_PARTS, NP * TP // WO_PARTS)
        late.append(pltpu.make_async_copy(wo_hbm.at[rows], wob16.at[rows], next(free)))
    for src, dst in ((w1_hbm, w1b16), (w3_hbm, w3b16)):
        late += retiled(src, dst, next(free), next(free))
    for f0, f1 in zip(W2_SPLIT[:-1], W2_SPLIT[1:]):
        rows = pl.ds(8 * f0, 8 * (f1 - f0))
        late.append(pltpu.make_async_copy(w2_hbm.at[rows], w2b16.at[rows], next(free)))

    def wait(copies):
        for c in copies:
            c.wait()

    def wait_late(n):
        late[n].wait()
        if n + IN_FLIGHT < len(late):
            late[n + IN_FLIGHT].start(priority=1)

    def set_lhs(x):
        d = x - jnp.sum(x, axis=1, keepdims=True) * (1.0 / D)
        xl[...] = _pack(d)
        var = jnp.sum(d * d, axis=1, keepdims=True) * (1.0 / D)
        rstd[...] = jnp.broadcast_to(lax.rsqrt(var + EPS), rstd.shape)

    def stage_q(i, s):
        for j in range(3):
            for t in range(DC):
                w = _tile(wqb[8 * t:8 * (t + 1), 3 * i + j])
                s["r"][j, t] = _mm(xl[:, 128 * t:128 * (t + 1)], w)

    def finish_q(s):
        for j in range(3):
            q = jnp.sum(s["r"][j], axis=0)
            s["q"][j] = _pack(_own_head(q, j) if j == 1 else q)

    def stage_k(i, s):
        for c in range(NC):
            u = (2 * c) % 8
            r = [_mm(s["q"][j], _tile(kb[pl.ds(TP * i + 8 * j, 8), c])) for j in range(3)]
            s["a"][2 * c:2 * c + 1, :] = r[0][u:u + 1]
            s["b"][2 * c:2 * c + 2, :] = r[1][u:u + 2]
            s["a"][2 * c + 1:2 * c + 2, :] = r[2][u + 1:u + 2]

    def softmax_lanes(s):
        z = (s["a"][...] + s["b"][...]).reshape(2 * NC // 8, 8, 128)
        z = z * (rstd[...] * DH ** -0.5)[None]
        m = _same_head(jnp.max(z, axis=0), jnp.maximum)
        e = jnp.exp(z - m[None])
        s["m"][0], s["m"][1] = m, _same_head(jnp.sum(e, axis=0), jnp.add)
        s["p"][...] = e.reshape(2 * NC, 128)

    def row_max(s):
        s["M"][...] = jnp.broadcast_to(jnp.max(s["m"][0], axis=1, keepdims=True), (8, 128))

    def stage_v(i, s, wide):
        for t0 in range(0, TP, V_GROUP):
            e = t0 // (TP // 2)
            lo, hi = [None] * V_GROUP, [None] * V_GROUP
            for c in range(NC):
                p = jnp.broadcast_to(s["p"][2 * c + e:2 * c + e + 1, :], (8, 128))
                for u in range(V_GROUP):
                    t, x = TP * i + t0 + u, c - (NC - WIDE)
                    w = vb[t, c]
                    if wide and x >= 0:
                        a, b = w, vx[t, x]
                    else:
                        a, b = w << 16, w & np.uint32(0xFFFF0000)
                        if x >= 0:
                            vb[t, c], vx[t, x] = a, b
                    a, b = pltpu.bitcast(a, F32) * p, pltpu.bitcast(b, F32) * p
                    lo[u] = a if c == 0 else lo[u] + a
                    hi[u] = b if c == 0 else hi[u] + b
            for u in range(V_GROUP):
                s["o"][pl.ds(16 * (t0 + u), 8, stride=2), :] = lo[u]
                s["o"][pl.ds(16 * (t0 + u) + 1, 8, stride=2), :] = hi[u]

    def weigh_lanes(s):
        f = jnp.exp(s["m"][0] - s["M"][...])
        s["l"][...] = f * s["m"][1]
        for e in range(2):
            rows = slice(e * DH, (e + 1) * DH)
            s["u"][rows, :] = s["o"][rows, :] * f[e:e + 1]

    def flip_o(s):
        s["L"][...] = jnp.broadcast_to(jnp.sum(s["l"][...], axis=1, keepdims=True), (8, 128))
        for j in range(0, 2 * DH, 128):
            s["u"][j:j + 128, :] = s["u"][j:j + 128, :].T

    def finish_o(i, s):
        scale = 1.0 / s["L"][...]
        for j in range(3):
            inv = _own_head(scale, j)
            o = jnp.sum(s["u"][128 * j:128 * (j + 1), :].reshape(16, 8, 128), axis=0)
            o = _same_head(o * (inv + pltpu.roll(inv, 1, 0)), jnp.add)
            ol[i, j] = _pack(o + pltpu.roll(o, 1, 0))

    def halves(ref, rows, c):
        return jnp.concatenate(
            [ref[rows, 4 * c:4 * c + 4, :], ref[rows, 20 + 4 * c:24 + 4 * c, :]], axis=1
        )

    def stage_wo_first(i):
        for j in range(3):
            rows = pl.ds(TP * i + 8 * j, 8)
            ws = [halves(wob, rows, c) for c in range(DC)]
            for c in range(DC):
                wob[rows, 8 * c:8 * c + 8, :] = ws[c]
                yb[c, 0] += _mm(ol[i + 3, j], _tile(ws[c]))

    def stage_wo(i):
        for b in range(3 * i, 3 * i + 3):
            for c in range(DC):
                r = _mm(ol[i + 3, b % 3], _tile(wob[8 * b:8 * b + 8, 8 * c:8 * c + 8, :]))
                yb[c, b // 8, b % 8:b % 8 + 1, :] = r[b % 8:b % 8 + 1]

    def ffn_up():
        for f in range(FC):
            gu = []
            for w in (w1b, w3b):
                acc = None
                for t in range(DC):
                    r = _mm(xl[:, 128 * t:128 * (t + 1)], _tile(w[8 * t:8 * (t + 1), f]))
                    acc = r if acc is None else acc + r
                gu.append(acc * rstd[...])
            g, u = gu
            hl[f] = _pack(g * (1.0 / (1.0 + jnp.exp(-g))) * u)

    def ffn_down(x, f0, f1):
        cols = [x[:, 128 * c:128 * (c + 1)] for c in range(DC)]
        for f in range(f0, f1):
            for c in range(DC):
                cols[c] = cols[c] + _mm(hl[f], _tile(halves(w2b, slice(8 * f, 8 * f + 8), c)))
        return jnp.concatenate(cols, axis=1)

    def loop(lo, hi, fn):
        def body(i, carry):
            fn(i)
            return carry

        lax.fori_loop(lo, hi, body, 0)

    wait(cp_x)
    x = jnp.broadcast_to(xb[...].astype(F32), (8, D))
    set_lhs(x)
    wait(cp_wq)

    def attend(n):
        i = NP - 1 - n
        for g, hi in enumerate(KV_SPLIT[:-1]):
            @pl.when(i == hi - 1)
            def _():
                wait(cp_kv[g])
                if g == len(cp_kv) - 2:
                    for c in late[:IN_FLIGHT]:
                        c.start(priority=1)

        s = slots[0]
        stage_q(i, s)
        finish_q(s)
        stage_k(i, s)
        softmax_lanes(s)
        stage_v(i, s, False)
        row_max(s)
        weigh_lanes(s)
        flip_o(s)
        finish_o(i + 3, s)

    loop(0, NP, attend)
    for c in range(DC):
        yb[c, 0] = x[:, 128 * c:128 * (c + 1)]

    def project(i):
        for n in range(WO_PARTS):
            pl.when(i == n * NP // WO_PARTS)(lambda: wait_late(n))
        stage_wo_first(i)

    loop(0, NP, project)
    x = jnp.concatenate([yb[c, 0] for c in range(DC)], axis=1)
    set_lhs(x)
    for name in "mMoulL":
        slots[1][name][...] = slots[0][name][...]
    for n in range(4):
        wait_late(WO_PARTS + n)
    ffn_up()
    for j, (f0, f1) in enumerate(zip(W2_SPLIT[:-1], W2_SPLIT[1:])):
        wait_late(WO_PARTS + 4 + j)
        x = ffn_down(x, f0, f1)

    set_lhs(x)

    def barrier():
        pl.semaphore_wait(fence, 0)

    def step(i, e, more=2):
        this, other = slots[e], slots[1 - e]
        finish_o(i, other)
        weigh_lanes(other)
        if more > 1:
            finish_q(other)
        if more > 0:
            softmax_lanes(other)
        stage_v(i, this, True)
        if more > 1:
            stage_k(i + 2, this)
            stage_q(jnp.minimum(i + 4, NP - 1), this)
        row_max(this)
        flip_o(this)

    def two_steps(n):
        step(2 * n, 0)
        barrier()
        step(2 * n + 1, 1)

    even, odd = slots
    for i, s in enumerate(slots):
        stage_q(i, s)
        finish_q(s)
    stage_k(0, even)
    softmax_lanes(even)
    stage_k(1, odd)
    stage_q(2, even)
    finish_q(even)
    stage_q(3, odd)
    loop(0, NP // 2 - 1, two_steps)
    step(NP - 2, 0, 1)
    for i in range(6):
        stage_wo(i)
    barrier()
    step(NP - 1, 1, 0)
    for i in range(6, NP - 4):
        stage_wo(i)
    barrier()
    finish_o(NP, odd)
    weigh_lanes(odd)
    for i, s in enumerate(slots, NP + 1):
        flip_o(s)
        finish_o(i, s)
    for i in range(NP - 4, NP):
        stage_wo(i)
    y = jnp.concatenate([jnp.sum(yb[c], axis=0) for c in range(DC)], axis=1)
    y = y + pltpu.roll(y, 1, 0)
    x = x + _same_head(y, jnp.add)
    set_lhs(x)
    ffn_up()
    x = ffn_down(x, 0, FC)
    o_ref[...] = x[0:1].astype(o_ref.dtype)


def _groups(w):
    r, c = w.shape
    return w.reshape(r // 16, 2, 8, c // 128, 128).transpose(0, 1, 3, 2, 4)


@jax.jit
def pallas_interleave_layers__sliding_block_cached__glu_gated_swiglu__decode_kernel(
    A_x: jax.Array,
    A_k_cache: jax.Array,
    A_v_cache: jax.Array,
    A_wq: jax.Array,
    A_wo: jax.Array,
    B_x: jax.Array,
    B_w1: jax.Array,
    B_w3: jax.Array,
    B_w2: jax.Array,
):
    del B_x

    def cache(c):
        return _groups(jnp.swapaxes(c, 2, 3).reshape(H * DH, SK))

    def flat(w):
        return _groups(w).reshape(w.shape[0] // 16, 2 * DC * 8, 128)

    slot = {
        "r": pltpu.VMEM((3, DC, 8, 128), F32),
        "q": pltpu.VMEM((3, 8, 128), U32),
        "a": pltpu.VMEM((2 * NC, 128), F32),
        "b": pltpu.VMEM((2 * NC, 128), F32),
        "m": pltpu.VMEM((2, 8, 128), F32),
        "p": pltpu.VMEM((2 * NC, 128), F32),
        "M": pltpu.VMEM((8, 128), F32),
        "o": pltpu.VMEM((2 * DH, 128), F32),
        "u": pltpu.VMEM((2 * DH, 128), F32),
        "l": pltpu.VMEM((8, 128), F32),
        "L": pltpu.VMEM((8, 128), F32),
        "y": pltpu.VMEM((3, 8, 128), U32),
    }
    out = pl.pallas_call(
        _kernel,
        out_shape=jax.ShapeDtypeStruct((1, D), A_x.dtype),
        in_specs=[pl.BlockSpec(memory_space=pl.ANY)] * 8,
        scratch_shapes=[
            pltpu.VMEM((1, D), BF16),
            [
                pltpu.VMEM((NP * TP, NC, 16, 128), BF16),
                pltpu.VMEM((NP * TP, NC, 16, 128), BF16),
                pltpu.VMEM((D // 16, H * DH // 128, 16, 128), BF16),
                pltpu.VMEM((H * DH // 16, 2 * DC * 8, 128), BF16),
                pltpu.VMEM((D // 16, FC, 16, 128), BF16),
                pltpu.VMEM((D // 16, FC, 16, 128), BF16),
                pltpu.VMEM((F // 16, 2 * DC * 8, 128), BF16),
            ],
            pltpu.VMEM((NP * TP, WIDE, 8, 128), U32),
            pltpu.VMEM((8, D), U32),
            pltpu.VMEM((8, 128), F32),
            pltpu.VMEM((NP + 3, 3, 8, 128), U32),
            pltpu.VMEM((DC, 3 * NP // 8, 8, 128), F32),
            pltpu.VMEM((FC, 8, 128), U32),
            pltpu.SemaphoreType.DMA((len(KV_SPLIT) + WO_PARTS + len(W2_SPLIT) + 4,)),
            pltpu.SemaphoreType.REGULAR(()),
            [slot] * 2,
        ],
        compiler_params=pltpu.CompilerParams(vmem_limit_bytes=128 * 1024 * 1024),
        name="interleave_decode",
    )(
        A_x.reshape(1, D),
        cache(A_k_cache),
        cache(A_v_cache),
        _groups(A_wq),
        flat(A_wo),
        _groups(B_w1),
        _groups(B_w3),
        flat(B_w2),
    )
    return out.reshape(1, 1, D)
```

```python
import jax
import jax.numpy as jnp
import numpy as np
from jax import lax
from jax.experimental import pallas as pl
from jax.experimental.pallas import tpu as pltpu

D = 640
H = 32
DH = 192
SK = 32768
W = min(4096, max(256, SK // 4))
F = 1536
EPS = 1e-5

NP = H // 2
NC = W // 128
TP = 2 * DH // 16
DC = D // 128
FC = F // 128
KV_SPLIT = (16, 12, 8, 4, 2, 1, 0)
WO_PARTS = 8
IN_FLIGHT = 3
W2_SPLIT = (0, 8, 11, 12)
LAG = 4
V_GROUP = 6
WIDE = 6

BF16 = jnp.bfloat16
F32 = jnp.float32
U32 = jnp.uint32


def _tile(words):
    return pltpu.bitcast(words.reshape(64, 128), BF16)


def _mm(lhs_words, tile):
    lhs = pltpu.bitcast(lhs_words, BF16)
    return jnp.dot(lhs, tile, preferred_element_type=F32)[:8]


def _pack(rows8):
    both = jnp.concatenate([rows8, rows8], axis=0).astype(BF16)
    return pltpu.bitcast(both, U32)


def _same_head(a, op):
    a = op(a, pltpu.roll(a, 2, 0))
    return op(a, pltpu.roll(a, 4, 0))


def _own_head(a, j):
    row = lax.broadcasted_iota(jnp.int32, a.shape, 0)
    col = lax.broadcasted_iota(jnp.int32, a.shape, 1)
    return jnp.where((row & 1) == ((col >> 6) + j >> 1), a, 0.0)


def _kernel(
    x_hbm, k_hbm, v_hbm, wq_hbm, wo_hbm, w1_hbm, w3_hbm, w2_hbm,
    o_ref,
    xb, big, vx, xl, rstd, ol, yb, hl, sems, fence, slots,
):
    kb16, vb16, wqb16, wob16, w1b16, w3b16, w2b16 = big
    kb, vb, wqb, wob, w1b, w3b, w2b = (r.bitcast(U32) for r in big)

    def retiled(src, dst, *sem):
        return [
            pltpu.make_async_copy(src.at[:, par], dst.at[:, :, pl.ds(8 * par, 8), :], sem[-par])
            for par in range(2)
        ]

    free = (sems.at[n] for n in range(sems.shape[0]))
    cp_x = [pltpu.make_async_copy(x_hbm, xb, next(free))]
    cp_wq = retiled(wq_hbm, wqb16, next(free))
    cp_kv = []
    for hi, lo in zip(KV_SPLIT[:-1], KV_SPLIT[1:]):
        rows, sem = pl.ds(TP * lo, TP * (hi - lo)), next(free)
        window = pl.ds(SK // 128 - NC, NC)
        cp_kv.append(
            retiled(k_hbm.at[rows, :, window], kb16.at[rows], sem)
            + retiled(v_hbm.at[rows, :, window], vb16.at[rows], sem)
        )
    for c in cp_wq + cp_x + sum(cp_kv, []):
        c.start()

    late = []
    for n in range(WO_PARTS):
        rows = pl.ds(n * NP * TP // WO_PARTS, NP * TP // WO_PARTS)
        late.append(pltpu.make_async_copy(wo_hbm.at[rows], wob16.at[rows], next(free)))
    for src, dst in ((w1_hbm, w1b16), (w3_hbm, w3b16)):
        late += retiled(src, dst, next(free), next(free))
    for f0, f1 in zip(W2_SPLIT[:-1], W2_SPLIT[1:]):
        rows = pl.ds(8 * f0, 8 * (f1 - f0))
        late.append(pltpu.make_async_copy(w2_hbm.at[rows], w2b16.at[rows], next(free)))

    def wait(copies):
        for c in copies:
            c.wait()

    def wait_late(n):
        late[n].wait()
        if n + IN_FLIGHT < len(late):
            late[n + IN_FLIGHT].start(priority=1)

    def set_lhs(x):
        d = x - jnp.sum(x, axis=1, keepdims=True) * (1.0 / D)
        xl[...] = _pack(d)
        var = jnp.sum(d * d, axis=1, keepdims=True) * (1.0 / D)
        rstd[...] = jnp.broadcast_to(lax.rsqrt(var + EPS), rstd.shape)

    def stage_q(i, s):
        for j in range(3):
            for t in range(DC):
                w = _tile(wqb[8 * t:8 * (t + 1), 3 * i + j])
                s["r"][j, t] = _mm(xl[:, 128 * t:128 * (t + 1)], w)

    def finish_q(s):
        for j in range(3):
            q = jnp.sum(s["r"][j], axis=0)
            s["q"][j] = _pack(_own_head(q, j) if j == 1 else q)

    def stage_k(i, s):
        for c in range(NC):
            u = (2 * c) % 8
            r = [_mm(s["q"][j], _tile(kb[pl.ds(TP * i + 8 * j, 8), c])) for j in range(3)]
            s["a"][2 * c:2 * c + 1, :] = r[0][u:u + 1]
            s["b"][2 * c:2 * c + 2, :] = r[1][u:u + 2]
            s["a"][2 * c + 1:2 * c + 2, :] = r[2][u + 1:u + 2]

    def softmax_lanes(s):
        z = (s["a"][...] + s["b"][...]).reshape(2 * NC // 8, 8, 128)
        z = z * (rstd[...] * DH ** -0.5)[None]
        m = _same_head(jnp.max(z, axis=0), jnp.maximum)
        e = jnp.exp(z - m[None])
        s["m"][0], s["m"][1] = m, _same_head(jnp.sum(e, axis=0), jnp.add)
        s["p"][...] = e.reshape(2 * NC, 128)

    def row_max(s):
        s["M"][...] = jnp.broadcast_to(jnp.max(s["m"][0], axis=1, keepdims=True), (8, 128))

    def stage_v(i, s, wide):
        for t0 in range(0, TP, V_GROUP):
            e = t0 // (TP // 2)
            lo, hi = [None] * V_GROUP, [None] * V_GROUP
            for c in range(NC):
                p = jnp.broadcast_to(s["p"][2 * c + e:2 * c + e + 1, :], (8, 128))
                for u in range(V_GROUP):
                    t, x = TP * i + t0 + u, c - (NC - WIDE)
                    w = vb[t, c]
                    if wide and x >= 0:
                        a, b = w, vx[t, x]
                    else:
                        a, b = w << 16, w & np.uint32(0xFFFF0000)
                        if x >= 0:
                            vb[t, c], vx[t, x] = a, b
                    a, b = pltpu.bitcast(a, F32) * p, pltpu.bitcast(b, F32) * p
                    lo[u] = a if c == 0 else lo[u] + a
                    hi[u] = b if c == 0 else hi[u] + b
            for u in range(V_GROUP):
                s["o"][pl.ds(16 * (t0 + u), 8, stride=2), :] = lo[u]
                s["o"][pl.ds(16 * (t0 + u) + 1, 8, stride=2), :] = hi[u]

    def weigh_lanes(s):
        f = jnp.exp(s["m"][0] - s["M"][...])
        s["l"][...] = f * s["m"][1]
        for e in range(2):
            rows = slice(e * DH, (e + 1) * DH)
            s["u"][rows, :] = s["o"][rows, :] * f[e:e + 1]

    def flip_o(s):
        s["L"][...] = jnp.broadcast_to(jnp.sum(s["l"][...], axis=1, keepdims=True), (8, 128))
        for j in range(0, 2 * DH, 128):
            s["u"][j:j + 128, :] = s["u"][j:j + 128, :].T

    def finish_o(i, s):
        scale = 1.0 / s["L"][...]
        for j in range(3):
            inv = _own_head(scale, j)
            o = jnp.sum(s["u"][128 * j:128 * (j + 1), :].reshape(16, 8, 128), axis=0)
            o = _same_head(o * (inv + pltpu.roll(inv, 1, 0)), jnp.add)
            ol[i, j] = _pack(o + pltpu.roll(o, 1, 0))

    def halves(ref, rows, c):
        return jnp.concatenate(
            [ref[rows, 4 * c:4 * c + 4, :], ref[rows, 20 + 4 * c:24 + 4 * c, :]], axis=1
        )

    def stage_wo_first(i):
        for j in range(3):
            rows = pl.ds(TP * i + 8 * j, 8)
            ws = [halves(wob, rows, c) for c in range(DC)]
            for c in range(DC):
                wob[rows, 8 * c:8 * c + 8, :] = ws[c]
                yb[c, 0] += _mm(ol[i + LAG, j], _tile(ws[c]))

    def stage_wo(i):
        for b in range(3 * i, 3 * i + 3):
            for c in range(DC):
                r = _mm(ol[i + LAG, b % 3], _tile(wob[8 * b:8 * b + 8, 8 * c:8 * c + 8, :]))
                yb[c, b // 8, b % 8:b % 8 + 1, :] = r[b % 8:b % 8 + 1]

    def ffn_up():
        for f in range(FC):
            gu = []
            for w in (w1b, w3b):
                acc = None
                for t in range(DC):
                    r = _mm(xl[:, 128 * t:128 * (t + 1)], _tile(w[8 * t:8 * (t + 1), f]))
                    acc = r if acc is None else acc + r
                gu.append(acc * rstd[...])
            g, u = gu
            hl[f] = _pack(g * (1.0 / (1.0 + jnp.exp(-g))) * u)

    def ffn_down(x, f0, f1):
        cols = [x[:, 128 * c:128 * (c + 1)] for c in range(DC)]
        for f in range(f0, f1):
            for c in range(DC):
                cols[c] = cols[c] + _mm(hl[f], _tile(halves(w2b, slice(8 * f, 8 * f + 8), c)))
        return jnp.concatenate(cols, axis=1)

    def loop(lo, hi, fn):
        def body(i, carry):
            fn(i)
            return carry

        lax.fori_loop(lo, hi, body, 0)

    wait(cp_x)
    x = jnp.broadcast_to(xb[...].astype(F32), (8, D))
    set_lhs(x)
    wait(cp_wq)

    def attend(n):
        i = NP - 1 - n
        for g, hi in enumerate(KV_SPLIT[:-1]):
            @pl.when(i == hi - 1)
            def _():
                wait(cp_kv[g])
                if g == len(cp_kv) - 2:
                    for c in late[:IN_FLIGHT]:
                        c.start(priority=1)

        s = slots[0]
        stage_q(i, s)
        finish_q(s)
        stage_k(i, s)
        softmax_lanes(s)
        stage_v(i, s, False)
        row_max(s)
        weigh_lanes(s)
        flip_o(s)
        finish_o(i + LAG, s)

    loop(0, NP, attend)
    for c in range(DC):
        yb[c, 0] = x[:, 128 * c:128 * (c + 1)]

    def project(i):
        for n in range(WO_PARTS):
            pl.when(i == n * NP // WO_PARTS)(lambda: wait_late(n))
        stage_wo_first(i)

    loop(0, NP, project)
    x = jnp.concatenate([yb[c, 0] for c in range(DC)], axis=1)
    set_lhs(x)
    for name in "moul":
        slots[1][name][...] = slots[0][name][...]
    for n in range(4):
        wait_late(WO_PARTS + n)
    ffn_up()
    for j, (f0, f1) in enumerate(zip(W2_SPLIT[:-1], W2_SPLIT[1:])):
        wait_late(WO_PARTS + 4 + j)
        x = ffn_down(x, f0, f1)

    set_lhs(x)

    def barrier():
        pl.semaphore_signal(fence, 1)
        pl.semaphore_wait(fence, 1)

    def step(i, e, more=2):
        this, other = slots[e], slots[1 - e]
        finish_o(i, this)
        weigh_lanes(this)
        softmax_lanes(this)
        if more > 1:
            finish_q(this)
        stage_v(i, this, True)
        if more > 0:
            stage_k(i + 1, other)
        if more > 1:
            stage_q(jnp.minimum(i + 3, NP - 1), other)
        row_max(other)
        flip_o(other)

    def two_steps(n):
        step(2 * n, 0)
        barrier()
        step(2 * n + 1, 1)

    even, odd = slots
    for i, s in enumerate(slots):
        stage_q(i, s)
        finish_q(s)
    stage_k(0, even)
    stage_q(2, even)
    loop(0, NP // 2 - 1, two_steps)
    step(NP - 2, 0, 1)
    stage_wo(0)
    barrier()
    step(NP - 1, 1, 0)
    for i in range(1, 9):
        stage_wo(i)
    barrier()
    row_max(odd)
    for i, s in enumerate(slots, NP):
        if s is odd:
            flip_o(s)
        finish_o(i, s)
        weigh_lanes(s)
        flip_o(s)
        finish_o(i + 2, s)
    for i in (9, 10, 11, 12, 14, 13, 15):
        stage_wo(i)
    y = jnp.concatenate([jnp.sum(yb[c], axis=0) for c in range(DC)], axis=1)
    y = y + pltpu.roll(y, 1, 0)
    x = x + _same_head(y, jnp.add)
    set_lhs(x)
    ffn_up()
    x = ffn_down(x, 0, FC)
    o_ref[...] = x[0:1].astype(o_ref.dtype)


def _groups(w):
    r, c = w.shape
    return w.reshape(r // 16, 2, 8, c // 128, 128).transpose(0, 1, 3, 2, 4)


@jax.jit
def pallas_interleave_layers__sliding_block_cached__glu_gated_swiglu__decode_kernel(
    A_x: jax.Array,
    A_k_cache: jax.Array,
    A_v_cache: jax.Array,
    A_wq: jax.Array,
    A_wo: jax.Array,
    B_x: jax.Array,
    B_w1: jax.Array,
    B_w3: jax.Array,
    B_w2: jax.Array,
):
    del B_x

    def cache(c):
        return _groups(jnp.swapaxes(c, 2, 3).reshape(H * DH, SK))

    def flat(w):
        return _groups(w).reshape(w.shape[0] // 16, 2 * DC * 8, 128)

    slot = {
        "r": pltpu.VMEM((3, DC, 8, 128), F32),
        "q": pltpu.VMEM((3, 8, 128), U32),
        "a": pltpu.VMEM((2 * NC, 128), F32),
        "b": pltpu.VMEM((2 * NC, 128), F32),
        "m": pltpu.VMEM((2, 8, 128), F32),
        "p": pltpu.VMEM((2 * NC, 128), F32),
        "M": pltpu.VMEM((8, 128), F32),
        "o": pltpu.VMEM((2 * DH, 128), F32),
        "u": pltpu.VMEM((2 * DH, 128), F32),
        "l": pltpu.VMEM((8, 128), F32),
        "L": pltpu.VMEM((8, 128), F32),
        "y": pltpu.VMEM((3, 8, 128), U32),
    }
    out = pl.pallas_call(
        _kernel,
        out_shape=jax.ShapeDtypeStruct((1, D), A_x.dtype),
        in_specs=[pl.BlockSpec(memory_space=pl.ANY)] * 8,
        scratch_shapes=[
            pltpu.VMEM((1, D), BF16),
            [
                pltpu.VMEM((NP * TP, NC, 16, 128), BF16),
                pltpu.VMEM((NP * TP, NC, 16, 128), BF16),
                pltpu.VMEM((D // 16, H * DH // 128, 16, 128), BF16),
                pltpu.VMEM((H * DH // 16, 2 * DC * 8, 128), BF16),
                pltpu.VMEM((D // 16, FC, 16, 128), BF16),
                pltpu.VMEM((D // 16, FC, 16, 128), BF16),
                pltpu.VMEM((F // 16, 2 * DC * 8, 128), BF16),
            ],
            pltpu.VMEM((NP * TP, WIDE, 8, 128), U32),
            pltpu.VMEM((8, D), U32),
            pltpu.VMEM((8, 128), F32),
            pltpu.VMEM((NP + LAG, 3, 8, 128), U32),
            pltpu.VMEM((DC, 3 * NP // 8, 8, 128), F32),
            pltpu.VMEM((FC, 8, 128), U32),
            pltpu.SemaphoreType.DMA((len(KV_SPLIT) + WO_PARTS + len(W2_SPLIT) + 4,)),
            pltpu.SemaphoreType.REGULAR(()),
            [slot] * 2,
        ],
        compiler_params=pltpu.CompilerParams(vmem_limit_bytes=128 * 1024 * 1024),
        name="interleave_decode",
    )(
        A_x.reshape(1, D),
        cache(A_k_cache),
        cache(A_v_cache),
        _groups(A_wq),
        flat(A_wo),
        _groups(B_w1),
        _groups(B_w3),
        flat(B_w2),
    )
    return out.reshape(1, 1, D)
```

```python
import jax
import jax.numpy as jnp
import numpy as np
from jax import lax
from jax.experimental import pallas as pl
from jax.experimental.pallas import tpu as pltpu

D = 640
H = 32
DH = 192
SK = 32768
W = min(4096, max(256, SK // 4))
F = 1536
EPS = 1e-5

NP = H // 2
NC = W // 128
TP = 2 * DH // 16
DC = D // 128
FC = F // 128
KV_SPLIT = (16, 12, 8, 4, 2, 1, 0)
WO_PARTS = 8
IN_FLIGHT = 3
W2_SPLIT = (0, 8, 11, 12)
LAG = 4
V_GROUP = 12
WIDE = 6

BF16 = jnp.bfloat16
F32 = jnp.float32
U32 = jnp.uint32


def _tile(words):
    return pltpu.bitcast(words.reshape(64, 128), BF16)


def _mm(lhs_words, tile):
    lhs = pltpu.bitcast(lhs_words, BF16)
    return jnp.dot(lhs, tile, preferred_element_type=F32)[:8]


def _pack(rows8):
    both = jnp.concatenate([rows8, rows8], axis=0).astype(BF16)
    return pltpu.bitcast(both, U32)


def _same_head(a, op):
    a = op(a, pltpu.roll(a, 2, 0))
    return op(a, pltpu.roll(a, 4, 0))


def _own_head(a, j):
    row = lax.broadcasted_iota(jnp.int32, a.shape, 0)
    col = lax.broadcasted_iota(jnp.int32, a.shape, 1)
    return jnp.where((row & 1) == ((col >> 6) + j >> 1), a, 0.0)


def _kernel(
    x_hbm, k_hbm, v_hbm, wq_hbm, wo_hbm, w1_hbm, w3_hbm, w2_hbm,
    o_ref,
    xb, big, vx, xl, rstd, ol, yb, hl, sems, fence, slots,
):
    kb16, vb16, wqb16, wob16, w1b16, w3b16, w2b16 = big
    kb, vb, wqb, wob, w1b, w3b, w2b = (r.bitcast(U32) for r in big)

    def retiled(src, dst, *sem):
        return [
            pltpu.make_async_copy(src.at[:, par], dst.at[:, :, pl.ds(8 * par, 8), :], sem[-par])
            for par in range(2)
        ]

    free = (sems.at[n] for n in range(sems.shape[0]))
    cp_x = [pltpu.make_async_copy(x_hbm, xb, next(free))]
    cp_wq = retiled(wq_hbm, wqb16, next(free))
    cp_kv = []
    for hi, lo in zip(KV_SPLIT[:-1], KV_SPLIT[1:]):
        rows, sem = pl.ds(TP * lo, TP * (hi - lo)), next(free)
        window = pl.ds(SK // 128 - NC, NC)
        cp_kv.append(
            retiled(k_hbm.at[rows, :, window], kb16.at[rows], sem)
            + retiled(v_hbm.at[rows, :, window], vb16.at[rows], sem)
        )
    for c in cp_wq + cp_x + sum(cp_kv, []):
        c.start()

    late = []
    for n in range(WO_PARTS):
        rows = pl.ds(n * NP * TP // WO_PARTS, NP * TP // WO_PARTS)
        late.append(pltpu.make_async_copy(wo_hbm.at[rows], wob16.at[rows], next(free)))
    for src, dst in ((w1_hbm, w1b16), (w3_hbm, w3b16)):
        late += retiled(src, dst, next(free), next(free))
    for f0, f1 in zip(W2_SPLIT[:-1], W2_SPLIT[1:]):
        rows = pl.ds(8 * f0, 8 * (f1 - f0))
        late.append(pltpu.make_async_copy(w2_hbm.at[rows], w2b16.at[rows], next(free)))

    def wait(copies):
        for c in copies:
            c.wait()

    def wait_late(n):
        late[n].wait()
        if n + IN_FLIGHT < len(late):
            late[n + IN_FLIGHT].start(priority=1)

    def set_lhs(x):
        d = x - jnp.sum(x, axis=1, keepdims=True) * (1.0 / D)
        xl[...] = _pack(d)
        var = jnp.sum(d * d, axis=1, keepdims=True) * (1.0 / D)
        rstd[...] = jnp.broadcast_to(lax.rsqrt(var + EPS), rstd.shape)

    def stage_q(i, s):
        for j in range(3):
            for t in range(DC):
                w = _tile(wqb[8 * t:8 * (t + 1), 3 * i + j])
                s["r"][j, t] = _mm(xl[:, 128 * t:128 * (t + 1)], w)

    def finish_q(s):
        for j in range(3):
            q = jnp.sum(s["r"][j], axis=0)
            s["q"][j] = _pack(_own_head(q, j) if j == 1 else q)

    def stage_k(i, s):
        for c in range(NC):
            u = (2 * c) % 8
            r = [_mm(s["q"][j], _tile(kb[pl.ds(TP * i + 8 * j, 8), c])) for j in range(3)]
            s["a"][2 * c:2 * c + 1, :] = r[0][u:u + 1]
            s["b"][2 * c:2 * c + 2, :] = r[1][u:u + 2]
            s["a"][2 * c + 1:2 * c + 2, :] = r[2][u + 1:u + 2]

    def softmax_lanes(s):
        z = (s["a"][...] + s["b"][...]).reshape(2 * NC // 8, 8, 128)
        z = z * (rstd[...] * DH ** -0.5)[None]
        m = _same_head(jnp.max(z, axis=0), jnp.maximum)
        e = jnp.exp(z - m[None])
        s["m"][0], s["m"][1] = m, _same_head(jnp.sum(e, axis=0), jnp.add)
        s["p"][...] = e.reshape(2 * NC, 128)

    def row_max(s):
        s["M"][...] = jnp.broadcast_to(jnp.max(s["m"][0], axis=1, keepdims=True), (8, 128))

    def stage_v(i, s, out, wide):
        for t0 in range(0, TP, V_GROUP):
            e = t0 // (TP // 2)
            lo, hi = [None] * V_GROUP, [None] * V_GROUP
            for c in range(NC):
                p = jnp.broadcast_to(s["p"][2 * c + e:2 * c + e + 1, :], (8, 128))
                for u in range(V_GROUP):
                    t, x = TP * i + t0 + u, c - (NC - WIDE)
                    w = vb[t, c]
                    if wide and x >= 0:
                        a, b = w, vx[t, x]
                    else:
                        a, b = w << 16, w & np.uint32(0xFFFF0000)
                        if x >= 0:
                            vb[t, c], vx[t, x] = a, b
                    a, b = pltpu.bitcast(a, F32) * p, pltpu.bitcast(b, F32) * p
                    lo[u] = a if c == 0 else lo[u] + a
                    hi[u] = b if c == 0 else hi[u] + b
            for u in range(V_GROUP):
                out[pl.ds(16 * (t0 + u), 8, stride=2), :] = lo[u]
                out[pl.ds(16 * (t0 + u) + 1, 8, stride=2), :] = hi[u]

    def weigh_lanes(s):
        f = jnp.exp(s["m"][0] - s["M"][...])
        s["f"][0], s["f"][1] = f, f * s["m"][1]

    def merge_lanes(s, parts):
        s["L"][...] = jnp.broadcast_to(jnp.sum(s["f"][1], axis=1, keepdims=True), (8, 128))
        for j in range(3):
            s["u"][j] = lax.dot_general(
                s["f"][0], parts[128 * j:128 * (j + 1), :], (((1,), (1,)), ((), ())),
                preferred_element_type=F32,
            )

    def finish_o(i, s):
        scale = 1.0 / s["L"][...]
        for j in range(3):
            o = _own_head(s["u"][j] * scale, j)
            ol[i, j] = _pack(o + pltpu.roll(o, 1, 0))

    def halves(ref, rows, c):
        return jnp.concatenate(
            [ref[rows, 4 * c:4 * c + 4, :], ref[rows, 20 + 4 * c:24 + 4 * c, :]], axis=1
        )

    def stage_wo_first(i):
        for j in range(3):
            rows = pl.ds(TP * i + 8 * j, 8)
            ws = [halves(wob, rows, c) for c in range(DC)]
            for c in range(DC):
                wob[rows, 8 * c:8 * c + 8, :] = ws[c]
                yb[c, 0] += _mm(ol[i + LAG, j], _tile(ws[c]))

    def stage_wo(i):
        for b in range(3 * i, 3 * i + 3):
            for c in range(DC):
                r = _mm(ol[i + LAG, b % 3], _tile(wob[8 * b:8 * b + 8, 8 * c:8 * c + 8, :]))
                yb[c, b // 8, b % 8:b % 8 + 1, :] = r[b % 8:b % 8 + 1]

    def ffn_up():
        for f in range(FC):
            gu = []
            for w in (w1b, w3b):
                acc = None
                for t in range(DC):
                    r = _mm(xl[:, 128 * t:128 * (t + 1)], _tile(w[8 * t:8 * (t + 1), f]))
                    acc = r if acc is None else acc + r
                gu.append(acc * rstd[...])
            g, u = gu
            hl[f] = _pack(g * (1.0 / (1.0 + jnp.exp(-g))) * u)

    def ffn_down(x, f0, f1):
        cols = [x[:, 128 * c:128 * (c + 1)] for c in range(DC)]
        for f in range(f0, f1):
            for c in range(DC):
                cols[c] = cols[c] + _mm(hl[f], _tile(halves(w2b, slice(8 * f, 8 * f + 8), c)))
        return jnp.concatenate(cols, axis=1)

    def loop(lo, hi, fn):
        def body(i, carry):
            fn(i)
            return carry

        lax.fori_loop(lo, hi, body, 0)

    wait(cp_x)
    x = jnp.broadcast_to(xb[...].astype(F32), (8, D))
    set_lhs(x)
    wait(cp_wq)

    def attend(n):
        i = NP - 1 - n
        for g, hi in enumerate(KV_SPLIT[:-1]):
            @pl.when(i == hi - 1)
            def _():
                wait(cp_kv[g])
                if g == len(cp_kv) - 2:
                    for c in late[:IN_FLIGHT]:
                        c.start(priority=1)

        s = slots[0]
        stage_q(i, s)
        finish_q(s)
        stage_k(i, s)
        softmax_lanes(s)
        stage_v(i, s, s["o"].at[0], False)
        row_max(s)
        weigh_lanes(s)
        merge_lanes(s, s["o"].at[0])
        finish_o(i + LAG, s)

    loop(0, NP, attend)
    for c in range(DC):
        yb[c, 0] = x[:, 128 * c:128 * (c + 1)]

    def project(i):
        for n in range(WO_PARTS):
            pl.when(i == n * NP // WO_PARTS)(lambda: wait_late(n))
        stage_wo_first(i)

    loop(0, NP, project)
    x = jnp.concatenate([yb[c, 0] for c in range(DC)], axis=1)
    set_lhs(x)
    for r in (slots[0]["o"], slots[1]["o"], slots[1]["m"], slots[1]["f"]):
        r[...] = jnp.ones(r.shape, F32)
    for n in range(4):
        wait_late(WO_PARTS + n)
    ffn_up()
    for j, (f0, f1) in enumerate(zip(W2_SPLIT[:-1], W2_SPLIT[1:])):
        wait_late(WO_PARTS + 4 + j)
        x = ffn_down(x, f0, f1)

    set_lhs(x)

    def barrier():
        pl.semaphore_signal(fence, 1)
        pl.semaphore_wait(fence, 1)

    def step(n, e, more=2):
        i, this, other = 2 * n + e, slots[e], slots[1 - e]
        finish_o(i, this)
        if more > 1:
            finish_q(this)
        weigh_lanes(this)
        softmax_lanes(this)
        stage_v(i, this, this["o"].at[n & 1], True)
        merge_lanes(other, other["o"].at[(n + e) & 1])
        if more > 0:
            stage_k(i + 1, other)
        if more > 1:
            stage_q(jnp.minimum(i + 3, NP - 1), other)
        row_max(other)

    def two_steps(n):
        step(n, 0)
        barrier()
        step(n, 1)

    even, odd = slots
    for i, s in enumerate(slots):
        stage_q(i, s)
        finish_q(s)
    stage_k(0, even)
    stage_q(2, even)
    loop(0, NP // 2 - 1, two_steps)
    step(NP // 2 - 1, 0, 1)
    stage_wo(0)
    barrier()
    step(NP // 2 - 1, 1, 0)
    for i in range(1, 9):
        stage_wo(i)
    barrier()
    row_max(odd)
    finish_o(NP, even)
    merge_lanes(odd, odd["o"].at[0])
    finish_o(NP + 1, odd)
    todo = iter(range(9, NP))
    for i, s in enumerate(slots, NP + 2):
        weigh_lanes(s)
        stage_wo(next(todo))
        stage_wo(next(todo))
        merge_lanes(s, s["o"].at[1])
        finish_o(i, s)
    for i in todo:
        stage_wo(i)
    y = jnp.concatenate([jnp.sum(yb[c], axis=0) for c in range(DC)], axis=1)
    y = y + pltpu.roll(y, 1, 0)
    x = x + _same_head(y, jnp.add)
    set_lhs(x)
    ffn_up()
    x = ffn_down(x, 0, FC)
    o_ref[...] = x[0:1].astype(o_ref.dtype)


def _groups(w):
    r, c = w.shape
    return w.reshape(r // 16, 2, 8, c // 128, 128).transpose(0, 1, 3, 2, 4)


@jax.jit
def pallas_interleave_layers__sliding_block_cached__glu_gated_swiglu__decode_kernel(
    A_x: jax.Array,
    A_k_cache: jax.Array,
    A_v_cache: jax.Array,
    A_wq: jax.Array,
    A_wo: jax.Array,
    B_x: jax.Array,
    B_w1: jax.Array,
    B_w3: jax.Array,
    B_w2: jax.Array,
):
    del B_x

    def cache(c):
        return _groups(jnp.swapaxes(c, 2, 3).reshape(H * DH, SK))

    def flat(w):
        return _groups(w).reshape(w.shape[0] // 16, 2 * DC * 8, 128)

    slot = {
        "r": pltpu.VMEM((3, DC, 8, 128), F32),
        "q": pltpu.VMEM((3, 8, 128), U32),
        "a": pltpu.VMEM((2 * NC, 128), F32),
        "b": pltpu.VMEM((2 * NC, 128), F32),
        "m": pltpu.VMEM((2, 8, 128), F32),
        "p": pltpu.VMEM((2 * NC, 128), F32),
        "M": pltpu.VMEM((8, 128), F32),
        "o": pltpu.VMEM((2, 2 * DH, 128), F32),
        "f": pltpu.VMEM((2, 8, 128), F32),
        "u": pltpu.VMEM((3, 8, 128), F32),
        "L": pltpu.VMEM((8, 128), F32),
    }
    out = pl.pallas_call(
        _kernel,
        out_shape=jax.ShapeDtypeStruct((1, D), A_x.dtype),
        in_specs=[pl.BlockSpec(memory_space=pl.ANY)] * 8,
        scratch_shapes=[
            pltpu.VMEM((1, D), BF16),
            [
                pltpu.VMEM((NP * TP, NC, 16, 128), BF16),
                pltpu.VMEM((NP * TP, NC, 16, 128), BF16),
                pltpu.VMEM((D // 16, H * DH // 128, 16, 128), BF16),
                pltpu.VMEM((H * DH // 16, 2 * DC * 8, 128), BF16),
                pltpu.VMEM((D // 16, FC, 16, 128), BF16),
                pltpu.VMEM((D // 16, FC, 16, 128), BF16),
                pltpu.VMEM((F // 16, 2 * DC * 8, 128), BF16),
            ],
            pltpu.VMEM((NP * TP, WIDE, 8, 128), U32),
            pltpu.VMEM((8, D), U32),
            pltpu.VMEM((8, 128), F32),
            pltpu.VMEM((NP + LAG, 3, 8, 128), U32),
            pltpu.VMEM((DC, 3 * NP // 8, 8, 128), F32),
            pltpu.VMEM((FC, 8, 128), U32),
            pltpu.SemaphoreType.DMA((len(KV_SPLIT) + WO_PARTS + len(W2_SPLIT) + 4,)),
            pltpu.SemaphoreType.REGULAR(()),
            [slot] * 2,
        ],
        compiler_params=pltpu.CompilerParams(vmem_limit_bytes=128 * 1024 * 1024),
        name="interleave_decode",
    )(
        A_x.reshape(1, D),
        cache(A_k_cache),
        cache(A_v_cache),
        _groups(A_wq),
        flat(A_wo),
        _groups(B_w1),
        _groups(B_w3),
        flat(B_w2),
    )
    return out.reshape(1, 1, D)
```
